```python
import jax
import jax.numpy as jnp

def _softmax(x, axis=-1):
    return jax.nn.softmax(x, axis=axis)

def _gelu(x):
    return jax.nn.gelu(x, approximate=True)

def _silu(x):
    return jax.nn.silu(x)

def _sigmoid(x):
    return jax.nn.sigmoid(x)

def _layernorm(x, axis=-1, eps=1e-05):
    m = jnp.mean(x, axis=axis, keepdims=True)
    v = jnp.var(x, axis=axis, keepdims=True)
    return (x - m) / jnp.sqrt(v + eps)

def _scatter_add(tgt, idx, src, axis=0):
    return tgt.at[idx].add(src)

def _segment_sum(src, seg, n):
    return jax.ops.segment_sum(src, seg, n)

class _Rng:

    def __init__(self, key):
        self._k = key

    def _next(self):
        self._k, sub = jax.random.split(self._k)
        return sub

    def normal(self, shape):
        return jax.random.normal(self._next(), shape, dtype=jnp.bfloat16)

    def randint(self, lo, hi, shape):
        return jax.random.randint(self._next(), shape, lo, hi, dtype=jnp.int32)

    def uniform(self, shape, lo=0.0, hi=1.0):
        return jax.random.uniform(self._next(), shape, jnp.bfloat16, lo, hi)

    def permutation(self, n):
        return jax.random.permutation(self._next(), n)
kernel_name = 'concat_heads__softmax_full_mha__memory_aug_recurrent_mem_tr__prompt'

def setup_inputs():
    _rng = _Rng(jax.random.key(int.from_bytes(__import__("os").urandom(4), "little")))
    _w = lambda a: (lambda t: t.astype(jnp.bfloat16) if jnp.issubdtype(t.dtype, jnp.floating) else t)(jnp.asarray(a))

    def _A_setup():
        B, S, D = (1, 2048, 1024)
        return {'x': _w((lambda *s: _rng.normal(s) * 0.05)(B, S, D)), 'wqkv': _w((lambda *s: _rng.normal(s) * 0.05)(D, 3 * D)), 'wo': _w((lambda *s: _rng.normal(s) * 0.05)(D, D))}
    _A_in = _A_setup()

    def _B_setup():
        B, S, Dm = (1, 2048, 1024)
        H, Dh = (32, 128)
        M, seg = (8, 32)
        seg = min(seg, S)
        S = S // seg * seg
        return {'x': _w((lambda *s: _rng.normal(s) * 0.05)(B, S, Dm)), 'mem0': _w((lambda *s: _rng.normal(s) * 0.05)(B, M, Dm)), 'Wq': _w((lambda *s: _rng.normal(s) * 0.05)(Dm, H, Dh) * Dm ** (-0.5)), 'Wk': _w((lambda *s: _rng.normal(s) * 0.05)(Dm, H, Dh) * Dm ** (-0.5)), 'Wv': _w((lambda *s: _rng.normal(s) * 0.05)(Dm, H, Dh) * Dm ** (-0.5)), 'Wo': _w((lambda *s: _rng.normal(s) * 0.05)(H, Dh, Dm) * (H * Dh) ** (-0.5)), 'seg_len': seg}
    _B_in = _B_setup()
    return {'A_x': _A_in['x'], 'A_wqkv': _A_in['wqkv'], 'A_wo': _A_in['wo'], 'B_x': _B_in['x'], 'B_mem0': _B_in['mem0'], 'B_Wq': _B_in['Wq'], 'B_Wk': _B_in['Wk'], 'B_Wv': _B_in['Wv'], 'B_Wo': _B_in['Wo'], 'B_seg_len': _B_in['seg_len']}

def reference(A_x, A_wqkv, A_wo, B_x, B_mem0, B_Wq, B_Wk, B_Wv, B_Wo, B_seg_len):

    def _A_ref(x, wqkv, wo):
        B, S, D = x.shape
        H = 32
        Dh = D // H
        qkv = (lambda x, *d: x.transpose(*d))((x @ wqkv).reshape(B, S, 3, H, Dh), 2, 0, 3, 1, 4)
        q, k, v = (qkv[0], qkv[1], qkv[2])
        scale = Dh ** (-0.5)
        scores = jnp.einsum('bhqd,bhkd->bhqk', q, k) * scale
        p = _softmax(scores, axis=-1)
        o = jnp.einsum('bhqk,bhkd->bhqd', p, v)
        return (lambda x, *d: x.transpose(*d))(o, 0, 2, 1, 3).reshape(B, S, D) @ wo

    def _B_ref(x, mem0, Wq, Wk, Wv, Wo, seg_len):
        B, S, Dm = x.shape
        H, Dh = (Wq.shape[1], Wq.shape[2])
        M = mem0.shape[1]
        scale = Dh ** (-0.5)
        n_seg = S // seg_len
        L = M + seg_len
        idx = jnp.arange(L)
        mask = (idx[:, None] < M) | (idx[:, None] >= idx[None, :])
        mem = mem0
        outs = []
        for s in range(n_seg):
            xs = x[:, s * seg_len:(s + 1) * seg_len, :].copy()
            h = jnp.concatenate([mem, xs], axis=1)
            q = jnp.einsum('btd,dhe->bhte', h, Wq)
            k = jnp.einsum('btd,dhe->bhte', h, Wk)
            v = jnp.einsum('btd,dhe->bhte', h, Wv)
            scores = jnp.einsum('bhqe,bhke->bhqk', q, k) * scale
            scores = jnp.where(mask[None, None], scores, -1000000000.0)
            p = _softmax(scores, axis=-1)
            o = jnp.einsum('bhqk,bhke->bhqe', p, v)
            o = jnp.einsum('bhte,hed->btd', o, Wo)
            mem = o[:, :M, :].copy()
            outs.append(o[:, M:, :])
        return jnp.concatenate(outs, axis=1)
    a = _A_ref(A_x, A_wqkv, A_wo)
    b = _B_ref(B_x, B_mem0, B_Wq, B_Wk, B_Wv, B_Wo, B_seg_len)
    return jnp.concatenate([a, b], axis=-1)
```

```python
import functools

import jax
import jax.numpy as jnp
from jax import lax
import jax.experimental.pallas as pl
import jax.experimental.pallas.tpu as pltpu

F32 = jnp.float32
BF16 = jnp.bfloat16
U32 = jnp.uint32
LOG2E = 1.4426950408889634
NT_DIMS = (((1,), (1,)), ((), ()))

A_HEADS = 32
TQ = 128
KB = 128
ROWS1 = 256


def _bf(words):
    return pltpu.bitcast(words, BF16)


def _words(x_f32):
    return pltpu.bitcast(x_f32.astype(BF16), U32)


def _kernel(
    xa_hbm, wqkv_hbm, woa_hbm, xb_hbm, mem0_hbm, wq_hbm, wk_hbm, wv_hbm, wob_hbm,
    out_hbm,
    xa_s, wqkv_s, woa_s, xb_s, mem0_s, wob_s, raw_s, wq_s, wk_s, wv_s,
    qt_s, k_s, vt_s, s0, s1, m0, m1, qs0, qs1, o_s,
    h_s, bq_s, bk_s, bv_s, bo_s, out_s,
    sem_x, sem_w, sem_raw, sem_rest, sem_out,
    *, S, D, HB, DHB, M, SEG,
):
    G = D // 128
    DHA = D // A_HEADS
    NJ = S // TQ
    NU = G * NJ
    L = M + SEG
    NR1 = S // ROWS1
    DCH = D // NR1
    SEG_PER_J = TQ // SEG

    def x_copy(r):
        return pltpu.make_async_copy(
            xa_hbm.at[pl.ds(r * ROWS1, ROWS1), :], xa_s.at[pl.ds(r * ROWS1, ROWS1), :], sem_x.at[r])

    def wqkv_copy(n):
        return pltpu.make_async_copy(wqkv_hbm.at[:, pl.ds(n * 128, 128)], wqkv_s.at[n], sem_w)

    def raw_copies(r, slot):
        return [
            pltpu.make_async_copy(w.at[pl.ds(r * DCH, DCH)], raw_s.at[slot, i], sem_raw.at[slot])
            for i, w in enumerate((wq_hbm, wk_hbm, wv_hbm))
        ]

    rest = (
        [pltpu.make_async_copy(woa_hbm.at[:, pl.ds(n * 128, 128)], woa_s.at[n], sem_rest) for n in range(D // 128)]
        + [pltpu.make_async_copy(wob_hbm.at[:, pl.ds(n * 128, 128)], wob_s.at[n], sem_rest) for n in range(D // 128)]
        + [pltpu.make_async_copy(xb_hbm, xb_s, sem_rest), pltpu.make_async_copy(mem0_hbm, mem0_s, sem_rest)]
    )

    x_copy(0).start()
    for n in range(3 * G):
        wqkv_copy(n).start()
    for r in range(1, NR1):
        x_copy(r).start()
    for c in raw_copies(0, 0):
        c.start()
    for c in rest:
        c.start()
    for n in range(3 * G):
        wqkv_copy(n).wait()

    wqkv_w = wqkv_s.bitcast(U32)
    woa_w = woa_s.bitcast(U32)
    wob_w = wob_s.bitcast(U32)

    q_mul = (DHA ** -0.5) * LOG2E
    sub8 = lax.broadcasted_iota(jnp.int32, (8, 128), 0)

    def relayout(slot, r):
        dp0 = r * (DCH // 2)
        for i, dst in enumerate((wq_s, wk_s, wv_s)):
            for dd in range(0, DCH, 16):
                ev, od = {}, {}
                for t in range(8):
                    a = pltpu.bitcast(raw_s[slot, i, dd + 2 * t], U32)
                    b = pltpu.bitcast(raw_s[slot, i, dd + 2 * t + 1], U32)
                    e = (a & U32(0xFFFF)) | (b << 16)
                    o = (a >> 16) | (b & U32(0xFFFF0000))
                    for half in range(HB // 16):
                        ev[half, t] = e[half * 8:(half + 1) * 8]
                        od[half, t] = o[half * 8:(half + 1) * 8]
                for par, src in ((0, ev), (1, od)):
                    for half in range(HB // 16):
                        v = [src[half, t] for t in range(8)]
                        for k in (1, 2, 4):
                            msk = (sub8 & k) == 0
                            nv = list(v)
                            for t in range(8):
                                if t & k == 0:
                                    x_, y_ = v[t], v[t + k]
                                    nv[t] = jnp.where(msk, x_, pltpu.roll(y_, k, 0))
                                    nv[t + k] = jnp.where(msk, pltpu.roll(x_, 8 - k, 0), y_)
                            v = nv
                        for t in range(8):
                            hh = 2 * (half * 8 + t) + par
                            dst[hh, pl.ds(pl.multiple_of(dp0 + dd // 2, 8), 8), :] = v[t]

    def phase1(r, carry):
        slot = r % 2
        x_copy(r).wait()
        for c in raw_copies(r, slot):
            c.wait()

        @pl.when(r + 1 < NR1)
        def _():
            for c in raw_copies(r + 1, 1 - slot):
                c.start()

        r0 = pl.multiple_of(r * ROWS1, ROWS1)
        xt = xa_s[pl.ds(r0, ROWS1), :]
        for g in range(G):
            q = jnp.dot(xt, _bf(wqkv_w[g]), preferred_element_type=F32) * q_mul
            qt_s[g, :, pl.ds(r0, ROWS1)] = _words(q.T)
            k = jnp.dot(xt, _bf(wqkv_w[G + g]), preferred_element_type=F32)
            k_s[g, pl.ds(pl.multiple_of(r * (ROWS1 // 2), ROWS1 // 2), ROWS1 // 2), :] = _words(k)
            v = jnp.dot(xt, _bf(wqkv_w[2 * G + g]), preferred_element_type=F32)
            vt_s[g, :, pl.ds(r0, ROWS1)] = _words(v.T)
        relayout(slot, r)
        return carry

    lax.fori_loop(0, NR1, phase1, 0)

    for c in rest:
        c.wait()

    S_ = (s0, s1)
    M_ = (m0, m1)
    QS = (qs0, qs1)
    qs0[...] = jnp.zeros_like(qs0)
    qs1[...] = jnp.zeros_like(qs1)

    def set_q(u, slot):
        g = u % G
        c0 = pl.multiple_of((u // G) * TQ, TQ)
        for h in range(4):
            QS[slot][h * 16:(h + 1) * 16, h * TQ:(h + 1) * TQ] = qt_s[g, h * 16:(h + 1) * 16, pl.ds(c0, TQ)]

    def a_step(u, slot):
        un = jnp.minimum(u + 1, NU - 1)
        g = u % G
        gn = un % G
        cur, nxt = slot, 1 - slot
        set_q(un, nxt)
        m = M_[cur][...]
        mrun = None
        l = [jnp.zeros((8, TQ), F32) for _ in range(4)]
        acc = [jnp.zeros((DHA, TQ), F32) for _ in range(4)]
        for kb in range(S // KB):
            kk = _bf(k_s[gn, kb * (KB // 2):(kb + 1) * (KB // 2), :])
            sn = jnp.dot(kk, _bf(QS[nxt][...]), preferred_element_type=F32)
            S_[nxt][kb * KB:(kb + 1) * KB, :] = sn
            mx = sn.reshape(KB // 8, 8, 4 * TQ).max(axis=0)
            mrun = mx if mrun is None else jnp.maximum(mrun, mx)
            for h in range(4):
                sc = S_[cur][kb * KB:(kb + 1) * KB, h * TQ:(h + 1) * TQ]
                p = jnp.exp2(sc.reshape(KB // 8, 8, TQ) - m[None, :, h * TQ:(h + 1) * TQ])
                l[h] = l[h] + p.sum(axis=0)
                pb = p.reshape(KB, TQ).astype(BF16)
                vt = _bf(vt_s[g, h * 16:(h + 1) * 16, kb * KB:(kb + 1) * KB])
                acc[h] = acc[h] + jnp.dot(vt, pb, preferred_element_type=F32)
        M_[nxt][...] = jnp.broadcast_to(jnp.max(mrun, axis=0, keepdims=True), (8, 4 * TQ))
        ot = jnp.concatenate(
            [acc[h] / jnp.sum(l[h], axis=0, keepdims=True) for h in range(4)], axis=0)
        o_s[g] = _words(ot.T)

    scale_b = DHB ** -0.5
    qi = lax.broadcasted_iota(jnp.int32, (L, L), 0)
    ki = lax.broadcasted_iota(jnp.int32, (L, L), 1)
    mask = (qi < M) | (qi >= ki)

    def b_step(s):
        r0 = pl.multiple_of(s * SEG, SEG)
        h_s[M:L, :] = xb_s[pl.ds(r0, SEG), :].astype(F32)
        hx = h_s[...]
        for h in range(HB):
            bq_s[h] = jnp.dot(hx, _bf(wq_s[h]), preferred_element_type=F32)
            bk_s[h] = jnp.dot(hx, _bf(wk_s[h]), preferred_element_type=F32)
            bv_s[h] = jnp.dot(hx, _bf(wv_s[h]), preferred_element_type=F32)
        hs = range(HB)
        ss = [lax.dot_general(bq_s[h].astype(BF16), bk_s[h].astype(BF16), NT_DIMS,
                              preferred_element_type=F32) * scale_b for h in hs]
        ss = [jnp.where(mask, s_, -1000000000.0) for s_ in ss]
        ms = [jnp.max(s_, axis=-1, keepdims=True) for s_ in ss]
        ps = [jnp.exp(s_ - m_) for s_, m_ in zip(ss, ms)]
        ls = [jnp.sum(p_, axis=-1, keepdims=True) for p_ in ps]
        os_ = [jnp.dot(p_.astype(BF16), bv_s[h].astype(BF16), preferred_element_type=F32)
               for p_, h in zip(ps, hs)]
        for h, o_, l_ in zip(hs, os_, ls):
            bo_s[:, h * DHB:(h + 1) * DHB] = (o_ / l_).astype(BF16).astype(F32)
        o = bo_s[...]
        a = jnp.concatenate(
            [jnp.dot(o, _bf(wob_w[n]), preferred_element_type=F32) for n in range(D // 128)], axis=1)
        ab = a.astype(BF16)
        out_s[pl.ds(r0, SEG), D:2 * D] = ab[M:L]
        h_s[0:M, :] = ab[0:M].astype(F32)

    h_s[0:M, :] = mem0_s[...].astype(F32)
    set_q(0, 0)
    sv = jnp.dot(_bf(k_s[0]), _bf(qs0[...]), preferred_element_type=F32)
    s0[...] = sv
    m0[...] = jnp.broadcast_to(jnp.max(sv, axis=0, keepdims=True), (8, 4 * TQ))

    def out_copy(j):
        rows = pl.ds(pl.multiple_of(j * TQ, TQ), TQ)
        return pltpu.make_async_copy(out_s.at[rows, :], out_hbm.at[rows, :], sem_out)

    def block(j, carry):
        def inner(i, c):
            b_step(j * SEG_PER_J + i)
            a_step(j * G + 2 * i, 0)
            a_step(j * G + 2 * i + 1, 1)
            return c
        lax.fori_loop(0, SEG_PER_J, inner, 0)
        r0 = pl.multiple_of(j * TQ, TQ)
        ob = jnp.concatenate([_bf(o_s[g]) for g in range(G)], axis=1)
        for n in range(D // 128):
            y = jnp.dot(ob, _bf(woa_w[n]), preferred_element_type=F32)
            out_s[pl.ds(r0, TQ), n * 128:(n + 1) * 128] = y.astype(BF16)
        out_copy(j).start()
        return carry

    lax.fori_loop(0, NJ, block, 0)
    for j in range(NJ):
        out_copy(j).wait()


@functools.partial(jax.jit, static_argnames=("B_seg_len",))
def pallas_concat_heads__softmax_full_mha__memory_aug_recurrent_mem_tr__prompt_kernel(
    A_x: jax.Array,
    A_wqkv: jax.Array,
    A_wo: jax.Array,
    B_x: jax.Array,
    B_mem0: jax.Array,
    B_Wq: jax.Array,
    B_Wk: jax.Array,
    B_Wv: jax.Array,
    B_Wo: jax.Array,
    B_seg_len: int,
):
    _, S, D = A_x.shape
    _, HB, DHB = B_Wq.shape
    M = B_mem0.shape[1]
    SEG = int(B_seg_len)
    L = M + SEG
    G = D // 128
    NR1 = S // ROWS1
    DCH = D // NR1
    assert 2 * SEG * 2 == TQ and G == 2 * (TQ // SEG)

    vm = pltpu.VMEM
    scratch = [
        vm((S, D), BF16),
        vm((3 * G, D, 128), BF16),
        vm((G, D, 128), BF16),
        vm((S, D), BF16),
        vm((M, D), BF16),
        vm((G, HB * DHB, 128), BF16),
        vm((2, 3, DCH, HB, DHB), BF16),
        vm((HB, D // 2, DHB), U32),
        vm((HB, D // 2, DHB), U32),
        vm((HB, D // 2, DHB), U32),
        vm((G, 64, S), U32),
        vm((G, S // 2, 128), U32),
        vm((G, 64, S), U32),
        vm((S, 4 * TQ), F32),
        vm((S, 4 * TQ), F32),
        vm((8, 4 * TQ), F32),
        vm((8, 4 * TQ), F32),
        vm((64, 4 * TQ), U32),
        vm((64, 4 * TQ), U32),
        vm((G, TQ // 2, 128), U32),
        vm((L, D), F32),
        vm((HB, L, DHB), F32),
        vm((HB, L, DHB), F32),
        vm((HB, L, DHB), F32),
        vm((L, HB * DHB), F32),
        vm((S, 2 * D), BF16),
        pltpu.SemaphoreType.DMA((NR1,)),
        pltpu.SemaphoreType.DMA,
        pltpu.SemaphoreType.DMA((2,)),
        pltpu.SemaphoreType.DMA,
        pltpu.SemaphoreType.DMA,
    ]
    any_spec = pl.BlockSpec(memory_space=pl.ANY)
    out = pl.pallas_call(
        functools.partial(_kernel, S=S, D=D, HB=HB, DHB=DHB, M=M, SEG=SEG),
        out_shape=jax.ShapeDtypeStruct((S, 2 * D), A_x.dtype),
        in_specs=[any_spec] * 9,
        out_specs=any_spec,
        scratch_shapes=scratch,
        compiler_params=pltpu.CompilerParams(vmem_limit_bytes=120 * 1024 * 1024),
        name="fused_mha_rmt",
    )(
        A_x.reshape(S, D), A_wqkv, A_wo, B_x.reshape(S, D), B_mem0.reshape(M, D),
        B_Wq, B_Wk, B_Wv, B_Wo.reshape(HB * DHB, D),
    )
    return out.reshape(1, S, 2 * D)
```

```python
import functools
import itertools

import jax
import jax.numpy as jnp
from jax import lax
import jax.experimental.pallas as pl
import jax.experimental.pallas.tpu as pltpu

F32 = jnp.float32
BF16 = jnp.bfloat16
U32 = jnp.uint32
LOG2E = 1.4426950408889634
NT_DIMS = (((1,), (1,)), ((), ()))

A_HEADS = 32
TQ = 128
KB = 128
ROWS1 = 256


def _bf(words):
    return pltpu.bitcast(words, BF16)


def _words(x_f32):
    return pltpu.bitcast(x_f32.astype(BF16), U32)


def _after(never, dep, val):
    return jnp.where(never, dep, val)


def _kernel(
    xa_hbm, wqkv_hbm, woa_hbm, xb_hbm, mem0_hbm, wq_hbm, wk_hbm, wv_hbm, wob_hbm,
    out_hbm,
    xa_s, wqkv_s, woa_s, xb_s, mem0_s, wob_s, raw_s, wq_s, wk_s, wv_s,
    qt_s, k_s, vt_s, s0, s1, m0, m1, qs0, qs1, o_s,
    h_s, bq_s, bk_s, bv_s, bo_s, out_s,
    sem_x, sem_w, sem_raw, sem_early, sem_xb, sem_woa, sem_out,
    *, S, D, HB, DHB, M, SEG,
):
    G = D // 128
    DHA = D // A_HEADS
    NJ = S // TQ
    NU = G * NJ
    L = M + SEG
    NR1 = S // ROWS1
    DCH = D // NR1
    SEG_PER_J = TQ // SEG

    def x_copy(r):
        return pltpu.make_async_copy(
            xa_hbm.at[pl.ds(r * ROWS1, ROWS1), :], xa_s.at[pl.ds(r * ROWS1, ROWS1), :], sem_x.at[r])

    WGRP = [(0, 4), (4, 8), (8, 16), (16, 24)]

    def wqkv_copy(grp):
        lo, hi = WGRP[grp]
        cols = pl.ds(lo * 128, (hi - lo) * 128)
        return pltpu.make_async_copy(wqkv_hbm.at[:, cols], wqkv_s.at[:, cols], sem_w.at[grp])

    def raw_copies(r):
        return [
            pltpu.make_async_copy(w.at[pl.ds(r * DCH, DCH)], raw_s.at[r % 2, i], sem_raw.at[r % 2])
            for i, w in enumerate((wq_hbm, wk_hbm, wv_hbm))
        ]

    def wob_copy(n):
        return pltpu.make_async_copy(wob_hbm.at[:, pl.ds(n * 128, 128)], wob_s.at[n], sem_early)

    xb_first = pltpu.make_async_copy(xb_hbm.at[pl.ds(0, TQ), :], xb_s.at[pl.ds(0, TQ), :], sem_early)
    xb_rest = pltpu.make_async_copy(xb_hbm.at[pl.ds(TQ, S - TQ), :], xb_s.at[pl.ds(TQ, S - TQ), :], sem_xb)
    mem0_copy = pltpu.make_async_copy(mem0_hbm, mem0_s, sem_early)
    woa_copy = pltpu.make_async_copy(woa_hbm, woa_s, sem_woa)
    assert NR1 == G

    wob_w = wob_s.bitcast(U32)

    q_mul = (DHA ** -0.5) * LOG2E
    sub8 = lax.broadcasted_iota(jnp.int32, (8, 128), 0)
    pieces = [(i, dd) for i in range(3) for dd in range(0, DCH, 16)]

    def relayout_piece(r, i, dd, gate=None, never=None):
        dst = (wq_s, wk_s, wv_s)[i]
        slot = r % 2
        rows = pl.ds(pl.multiple_of(r * (DCH // 2) + dd // 2, 8), 8)
        ev, od = {}, {}
        for t in range(8):
            a = pltpu.bitcast(raw_s[slot, i, dd + 2 * t], U32)
            b = pltpu.bitcast(raw_s[slot, i, dd + 2 * t + 1], U32)
            if gate is not None:
                a = _after(jnp.concatenate([never] * (HB // 16), axis=0),
                           jnp.concatenate([gate] * (HB // 16), axis=0), a)
            e = (a & U32(0xFFFF)) | (b << 16)
            o = (a >> 16) | (b & U32(0xFFFF0000))
            for half in range(HB // 16):
                ev[half, t] = e[half * 8:(half + 1) * 8]
                od[half, t] = o[half * 8:(half + 1) * 8]
        for par, src in ((0, ev), (1, od)):
            for half in range(HB // 16):
                v = [src[half, t] for t in range(8)]
                for k in (1, 2, 4):
                    msk = (sub8 & k) == 0
                    nv = list(v)
                    for t in range(8):
                        if t & k == 0:
                            x_, y_ = v[t], v[t + k]
                            nv[t] = jnp.where(msk, x_, pltpu.roll(y_, k, 0))
                            nv[t + k] = jnp.where(msk, pltpu.roll(x_, 8 - k, 0), y_)
                    v = nv
                for t in range(8):
                    dst[2 * (half * 8 + t) + par, rows, :] = v[t]
        return dst[HB - 1, rows, :]

    def qkv_dots(r, never=None, hooks=None):
        r0 = pl.multiple_of(r * ROWS1, ROWS1)
        xt = xa_s[pl.ds(r0, ROWS1), :]
        dep = gate = None
        for n in range(3 * G):
            if hooks and n in hooks:
                hooks[n]()
            part, g = n // G, n % G
            w = wqkv_s[:, n * 128:(n + 1) * 128]
            if dep is not None:
                w = jnp.concatenate([_bf(_after(never, dep, pltpu.bitcast(w[0:16], U32))), w[16:]], axis=0)
            y = jnp.dot(xt, w, preferred_element_type=F32)
            if never is not None:
                dep = relayout_piece(r - 1, *pieces[n], gate=gate, never=never)
            gate = pltpu.bitcast(y[0:8], U32)
            if part == 0:
                qt_s[g, :, pl.ds(r0, ROWS1)] = _words((y * q_mul).T)
            elif part == 1:
                k_s[g, pl.ds(pl.multiple_of(r * (ROWS1 // 2), ROWS1 // 2), ROWS1 // 2), :] = _words(y)
            else:
                vt_s[g, :, pl.ds(r0, ROWS1)] = _words(y.T)

    with jax.named_scope('first'):
        x_copy(0).start()
        wqkv_copy(0).start()
        x_copy(0).wait()
        wqkv_copy(0).wait()
        wqkv_copy(1).start()

        def hook(k):
            def run():
                wqkv_copy(k).wait()
                if k + 1 < len(WGRP):
                    wqkv_copy(k + 1).start()
                else:
                    for c in raw_copies(0) + [x_copy(1), wob_copy(0), xb_first, mem0_copy]:
                        c.start()
            return run

        qkv_dots(0, hooks={WGRP[k][0]: hook(k) for k in range(1, len(WGRP))})

    def phase1(r, carry):
        x_copy(r).wait()
        for c in raw_copies(r - 1):
            c.wait()
        for c in raw_copies(r) + [wob_copy(r)]:
            c.start()

        @pl.when(r + 1 < NR1)
        def _():
            x_copy(r + 1).start()

        qkv_dots(r, jnp.full((8, 128), r, jnp.int32) < 0)
        return r

    with jax.named_scope('phase1'):
        last_r = lax.fori_loop(1, NR1, phase1, 0)

    with jax.named_scope('restwait'):
        for c in raw_copies(NR1 - 1):
            c.wait()
        for c in [wob_copy(n) for n in range(G)] + [xb_first, mem0_copy]:
            c.wait()
        xb_rest.start()
        woa_copy.start()

    S_ = (s0, s1)
    M_ = (m0, m1)
    QS = (qs0, qs1)
    qs0[...] = jnp.zeros_like(qs0)
    qs1[...] = jnp.zeros_like(qs1)

    def set_q(u, slot):
        g = u % G
        c0 = pl.multiple_of((u // G) * TQ, TQ)
        for h in range(4):
            QS[slot][h * 16:(h + 1) * 16, h * TQ:(h + 1) * TQ] = qt_s[g, h * 16:(h + 1) * 16, pl.ds(c0, TQ)]

    def scores_block(g, slot, kb, kw=None):
        kw = k_s[g, kb * (KB // 2):(kb + 1) * (KB // 2), :] if kw is None else kw
        sn = jnp.dot(_bf(kw), _bf(QS[slot][...]), preferred_element_type=F32)
        S_[slot][kb * KB:(kb + 1) * KB, :] = sn
        return sn.reshape(KB // 8, 8, 4 * TQ).max(axis=0)

    def finish_max(mrun, slot):
        M_[slot][...] = jnp.broadcast_to(jnp.max(mrun, axis=0, keepdims=True), (8, 4 * TQ))

    def a_slots(u, slot, never):
        un = jnp.minimum(u + 1, NU - 1)
        g = u % G
        cur, nxt = slot, 1 - slot
        set_q(un, nxt)
        m = M_[cur][...]
        mrun = None
        deps = {}
        l = [jnp.zeros((8, TQ), F32) for _ in range(4)]
        acc = [jnp.zeros((DHA, TQ), F32) for _ in range(4)]
        for kb in range(S // KB):
            mx = scores_block(un % G, nxt, kb)
            mrun = mx if mrun is None else jnp.maximum(mrun, mx)
            deps[kb] = mx
            for h in range(4):
                cols = slice(h * TQ, (h + 1) * TQ)
                mh = m[:, cols]
                if kb - 1 in deps:
                    mh = _after(never, deps[kb - 1][:, cols], mh)
                sc = S_[cur][kb * KB:(kb + 1) * KB, cols]
                p = jnp.exp2(sc.reshape(KB // 8, 8, TQ) - mh[None])
                l[h] = l[h] + p.sum(axis=0)
                vt = _bf(vt_s[g, h * 16:(h + 1) * 16, kb * KB:(kb + 1) * KB])
                acc[h] = acc[h] + jnp.dot(vt, p.reshape(KB, TQ).astype(BF16), preferred_element_type=F32)
            if kb < S // KB - 1:
                yield
        finish_max(mrun, nxt)
        ot = jnp.concatenate(
            [acc[h] / jnp.sum(l[h], axis=0, keepdims=True) for h in range(4)], axis=0)
        o_s[g] = _words(ot.T)
        yield

    scale_b = DHB ** -0.5
    qi = lax.broadcasted_iota(jnp.int32, (L, L), 0)
    ki = lax.broadcasted_iota(jnp.int32, (L, L), 1)
    mask = (qi < M) | (qi >= ki)

    def b_qkv(h):
        hx = h_s[...]
        bq_s[h] = jnp.dot(hx, _bf(wq_s[h]), preferred_element_type=F32)
        bk_s[h] = jnp.dot(hx, _bf(wk_s[h]), preferred_element_type=F32)
        bv_s[h] = jnp.dot(hx, _bf(wv_s[h]), preferred_element_type=F32)

    def b_scores(h):
        return lax.dot_general(bq_s[h], bk_s[h].astype(BF16), NT_DIMS, preferred_element_type=F32) * scale_b

    def b_softmax_pv(h, s_):
        s_ = jnp.where(mask, s_, -1000000000.0)
        m_ = jnp.max(s_, axis=-1, keepdims=True)
        p_ = jnp.exp(s_ - m_)
        l_ = jnp.sum(p_, axis=-1, keepdims=True)
        o_ = jnp.dot(p_, bv_s[h].astype(BF16), preferred_element_type=F32)
        r_ = pltpu.reciprocal(l_, approx=True)
        r_ = r_ * (2.0 - l_ * r_)
        bo_s[:, h * DHB:(h + 1) * DHB] = o_ * r_

    def fused_step(s, u0):
        never = jnp.full((8, TQ), s, jnp.int32) < 0
        a_iter = itertools.chain(a_slots(u0, 0, never), a_slots(u0 + 1, 1, never))
        AQ = 29
        TAIL = ("S", "A", "A", "P", "A", "P")
        LS, LP = 1, 2
        n_a = 0
        r0 = pl.multiple_of(s * SEG, SEG)
        h_s[M:L, :] = xb_s[pl.ds(r0, SEG), :].astype(F32)
        sc, ns, npv = {}, 0, 0
        for t in range(HB):
            b_qkv(t)
            if (t + 1) * AQ // HB > t * AQ // HB:
                next(a_iter); n_a += 1
            if t >= LS:
                sc[ns] = b_scores(ns); ns += 1
            if t >= LP:
                b_softmax_pv(npv, sc.pop(npv)); npv += 1
        for tok in TAIL:
            if tok == "A":
                next(a_iter); n_a += 1
            elif tok == "S":
                sc[ns] = b_scores(ns); ns += 1
            else:
                b_softmax_pv(npv, sc.pop(npv)); npv += 1
        assert ns == HB and npv == HB
        rem = 32 - n_a
        mem = []
        for n in range(G):
            a = jnp.dot(bo_s[...], _bf(wob_w[n]), preferred_element_type=F32)
            out_s[pl.ds(r0, SEG), D + n * 128:D + (n + 1) * 128] = a[M:L].astype(BF16)
            mem.append(a[0:M])
            for _ in range((n + 1) * rem // G - n * rem // G):
                next(a_iter); n_a += 1
        assert n_a == 32
        h_s[0:M, :] = jnp.concatenate(mem, axis=1)

    h_s[0:M, :] = mem0_s[...].astype(F32)
    set_q(0, 0)
    never0 = jnp.full((8, 128), last_r, jnp.int32) < 0
    mrun = None
    npc = len(pieces)
    nkb = S // KB
    dep = gate = None
    for kb in range(nkb):
        kw = k_s[0, kb * (KB // 2):(kb + 1) * (KB // 2), :]
        if dep is not None:
            kw = jnp.concatenate([_after(never0, dep, kw[0:8]), kw[8:]], axis=0)
        mx = scores_block(0, 0, kb, kw)
        mrun = mx if mrun is None else jnp.maximum(mrun, mx)
        for t in range(kb * npc // nkb, (kb + 1) * npc // nkb):
            dep = relayout_piece(NR1 - 1, *pieces[t], gate=gate, never=never0)
        gate = pltpu.bitcast(mx[:, 0:128], U32)
    finish_max(mrun, 0)

    def out_copy(j):
        rows = pl.ds(pl.multiple_of(j * TQ, TQ), TQ)
        return pltpu.make_async_copy(out_s.at[rows, :], out_hbm.at[rows, :], sem_out)

    def block(j, carry):
        @pl.when(j == 1)
        def _():
            xb_rest.wait()

        def inner(i, c):
            fused_step(j * SEG_PER_J + i, j * G + 2 * i)
            return c

        with jax.named_scope('inner'):
            lax.fori_loop(0, SEG_PER_J, inner, 0)

        @pl.when(j == 0)
        def _():
            woa_copy.wait()

        r0 = pl.multiple_of(j * TQ, TQ)
        ob = jnp.concatenate([_bf(o_s[g]) for g in range(G)], axis=1)
        for n in range(G):
            y = jnp.dot(ob, woa_s[:, n * 128:(n + 1) * 128], preferred_element_type=F32)
            out_s[pl.ds(r0, TQ), n * 128:(n + 1) * 128] = y.astype(BF16)
        out_copy(j).start()
        return carry

    with jax.named_scope('main'):
        lax.fori_loop(0, NJ, block, 0)
    for j in range(NJ):
        out_copy(j).wait()


@functools.partial(jax.jit, static_argnames=("B_seg_len",))
def pallas_concat_heads__softmax_full_mha__memory_aug_recurrent_mem_tr__prompt_kernel(
    A_x: jax.Array,
    A_wqkv: jax.Array,
    A_wo: jax.Array,
    B_x: jax.Array,
    B_mem0: jax.Array,
    B_Wq: jax.Array,
    B_Wk: jax.Array,
    B_Wv: jax.Array,
    B_Wo: jax.Array,
    B_seg_len: int,
):
    _, S, D = A_x.shape
    _, HB, DHB = B_Wq.shape
    M = B_mem0.shape[1]
    SEG = int(B_seg_len)
    L = M + SEG
    G = D // 128
    NR1 = S // ROWS1
    DCH = D // NR1
    assert 4 * SEG == TQ and G == 2 * (TQ // SEG)

    vm = pltpu.VMEM
    scratch = [
        vm((S, D), BF16),
        vm((D, 3 * D), BF16),
        vm((D, D), BF16),
        vm((S, D), BF16),
        vm((M, D), BF16),
        vm((G, HB * DHB, 128), BF16),
        vm((2, 3, DCH, HB, DHB), BF16),
        vm((HB, D // 2, DHB), U32),
        vm((HB, D // 2, DHB), U32),
        vm((HB, D // 2, DHB), U32),
        vm((G, 64, S), U32),
        vm((G, S // 2, 128), U32),
        vm((G, 64, S), U32),
        vm((S, 4 * TQ), F32),
        vm((S, 4 * TQ), F32),
        vm((8, 4 * TQ), F32),
        vm((8, 4 * TQ), F32),
        vm((64, 4 * TQ), U32),
        vm((64, 4 * TQ), U32),
        vm((G, TQ // 2, 128), U32),
        vm((L, D), F32),
        vm((HB, L, DHB), F32),
        vm((HB, L, DHB), F32),
        vm((HB, L, DHB), F32),
        vm((L, HB * DHB), F32),
        vm((S, 2 * D), BF16),
        pltpu.SemaphoreType.DMA((NR1,)),
        pltpu.SemaphoreType.DMA((4,)),
        pltpu.SemaphoreType.DMA((2,)),
        pltpu.SemaphoreType.DMA,
        pltpu.SemaphoreType.DMA,
        pltpu.SemaphoreType.DMA,
        pltpu.SemaphoreType.DMA,
    ]
    any_spec = pl.BlockSpec(memory_space=pl.ANY)
    out = pl.pallas_call(
        functools.partial(_kernel, S=S, D=D, HB=HB, DHB=DHB, M=M, SEG=SEG),
        out_shape=jax.ShapeDtypeStruct((S, 2 * D), A_x.dtype),
        in_specs=[any_spec] * 9,
        out_specs=any_spec,
        scratch_shapes=scratch,
        compiler_params=pltpu.CompilerParams(vmem_limit_bytes=120 * 1024 * 1024),
        name="fused_mha_rmt",
    )(
        A_x.reshape(S, D), A_wqkv, A_wo, B_x.reshape(S, D), B_mem0.reshape(M, D),
        B_Wq, B_Wk, B_Wv, B_Wo.reshape(HB * DHB, D),
    )
    return out.reshape(1, S, 2 * D)
```

```python
import functools
import itertools

import jax
import jax.numpy as jnp
from jax import lax
import jax.experimental.pallas as pl
import jax.experimental.pallas.tpu as pltpu

F32 = jnp.float32
BF16 = jnp.bfloat16
U32 = jnp.uint32
LOG2E = 1.4426950408889634
NT_DIMS = (((1,), (1,)), ((), ()))

A_HEADS = 32
TQ = 128
KB = 128
ROWS0 = 512
ROWS1 = 256


def _bf(words):
    return pltpu.bitcast(words, BF16)


def _words(x_f32):
    return pltpu.bitcast(x_f32.astype(BF16), U32)


def _after(never, dep, val):
    return jnp.where(never, dep, val)


def _kernel(
    xa_hbm, wqkv_hbm, woa_hbm, xb_hbm, mem0_hbm, wq_hbm, wk_hbm, wv_hbm, wob_hbm,
    out_hbm,
    xa_s, wqkv_s, woa_s, xb_s, mem0_s, wob_s, raw_s, wb_s,
    qt_s, k_s, vt_s, s0, s1, m0, m1, qs0, qs1, o_s,
    h_s, bq_s, bk_s, bv_s, bo_s, out_s,
    sem_x, sem_w, sem_raw, sem_early, sem_xb, sem_woa, sem_out,
    *, S, D, HB, DHB, M, SEG,
):
    G = D // 128
    DHA = D // A_HEADS
    NJ = S // TQ
    NU = G * NJ
    L = M + SEG
    NR1 = (S - ROWS0) // ROWS1
    DCH = D // 2
    assert NR1 == 6
    SEG_PER_J = TQ // SEG

    x_first = pltpu.make_async_copy(xa_hbm.at[pl.ds(0, ROWS0), :], xa_s.at[pl.ds(0, ROWS0), :], sem_x.at[NR1])

    def x_copy(r):
        rows = pl.ds(ROWS0 + r * ROWS1, ROWS1)
        return pltpu.make_async_copy(xa_hbm.at[rows, :], xa_s.at[rows, :], sem_x.at[r])

    WGRP = [(0, 2), (2, 6), (6, 14), (14, 24)]

    def wqkv_copy(grp):
        lo, hi = WGRP[grp]
        cols = pl.ds(lo * 128, (hi - lo) * 128)
        return pltpu.make_async_copy(wqkv_hbm.at[:, cols], wqkv_s.at[:, cols], sem_w.at[grp])

    def raw_copy(i, half, slot):
        w = (wq_hbm, wk_hbm, wv_hbm)[i]
        return pltpu.make_async_copy(w.at[pl.ds(half * DCH, DCH)], raw_s.at[slot], sem_raw.at[slot])

    def start_raw(c):
        for i in range(3):
            @pl.when(c // 2 == i)
            def _():
                raw_copy(i, c % 2, c % 2).start()

    def wait_raw(c):
        raw_copy(0, 0, c % 2).wait()

    def wob_copy(n):
        return pltpu.make_async_copy(wob_hbm.at[:, pl.ds(n * 128, 128)], wob_s.at[n], sem_early)

    xb_first = pltpu.make_async_copy(xb_hbm.at[pl.ds(0, TQ), :], xb_s.at[pl.ds(0, TQ), :], sem_early)
    xb_rest = pltpu.make_async_copy(xb_hbm.at[pl.ds(TQ, S - TQ), :], xb_s.at[pl.ds(TQ, S - TQ), :], sem_xb)
    mem0_copy = pltpu.make_async_copy(mem0_hbm, mem0_s, sem_early)
    woa_copy = pltpu.make_async_copy(woa_hbm, woa_s, sem_woa)

    wob_w = wob_s.bitcast(U32)

    q_mul = (DHA ** -0.5) * LOG2E
    sub8 = lax.broadcasted_iota(jnp.int32, (8, 128), 0)
    pieces = [(dd, half) for dd in range(0, DCH, 16) for half in range(HB // 16)]

    def relayout_piece(c, dd, half, gate=None, never=None):
        slot = c % 2
        rows = pl.ds(pl.multiple_of(slot * (DCH // 2) + dd // 2, 8), 8)
        wsel = c // 2
        ev, od = [], []
        for t in range(8):
            a = pltpu.bitcast(raw_s[slot, dd + 2 * t, half * 16:(half + 1) * 16, :], U32)
            b = pltpu.bitcast(raw_s[slot, dd + 2 * t + 1, half * 16:(half + 1) * 16, :], U32)
            if gate is not None:
                a = _after(never, gate, a)
            ev.append((a & U32(0xFFFF)) | (b << 16))
            od.append((a >> 16) | (b & U32(0xFFFF0000)))
        for par, v in ((0, ev), (1, od)):
            for k in (1, 2, 4):
                msk = (sub8 & k) == 0
                nv = list(v)
                for t in range(8):
                    if t & k == 0:
                        x_, y_ = v[t], v[t + k]
                        nv[t] = jnp.where(msk, x_, pltpu.roll(y_, k, 0))
                        nv[t + k] = jnp.where(msk, pltpu.roll(x_, 8 - k, 0), y_)
                v = nv
            for t in range(8):
                wb_s[wsel, 2 * (half * 8 + t) + par, rows, :] = v[t]
        return wb_s[wsel, half * 16 + 15, rows, :]

    def qkv_dots(r0, rows, chunk=None, never=None, hooks=None):
        xt = xa_s[pl.ds(r0, rows), :]
        deps = {}
        gate = None
        npc = len(pieces)
        LAG, GSTEP = 2, 80
        for n in range(3 * G):
            if hooks and n in hooks:
                hooks[n]()
            part, g = n // G, n % G
            w = wqkv_s[:, n * 128:(n + 1) * 128]
            if n - LAG in deps:
                w = jnp.concatenate([_bf(_after(never, deps[n - LAG], pltpu.bitcast(w[0:16], U32))), w[16:]], axis=0)
            y = jnp.dot(xt, w, preferred_element_type=F32)
            if chunk is not None:
                lo, hi = n * npc // (3 * G), (n + 1) * npc // (3 * G)
                for t in range(lo, hi):
                    gt = None if gate is None else gate[(t - lo) * GSTEP:(t - lo) * GSTEP + 8]
                    deps[n] = relayout_piece(chunk, *pieces[t], gate=gt, never=never)
            gate = pltpu.bitcast(y, U32)
            if part == 0:
                qt_s[g, :, pl.ds(r0, rows)] = _words((y * q_mul).T)
            elif part == 1:
                k_s[g, pl.ds(pl.multiple_of(r0 // 2, rows // 2), rows // 2), :] = _words(y)
            else:
                vt_s[g, :, pl.ds(r0, rows)] = _words(y.T)

    with jax.named_scope('first'):
        x_first.start()
        wqkv_copy(0).start()
        x_first.wait()
        wqkv_copy(0).wait()
        wqkv_copy(1).start()
        wqkv_copy(2).start()

        def hook(k):
            def run():
                wqkv_copy(k).wait()
                if k + 2 < len(WGRP):
                    wqkv_copy(k + 2).start()
                elif k + 2 == len(WGRP):
                    raw_copy(0, 0, 0).start()
                else:
                    for c in [x_copy(0), wob_copy(6), wob_copy(7), xb_first, mem0_copy]:
                        c.start()
            return run

        qkv_dots(0, ROWS0, hooks={WGRP[k][0]: hook(k) for k in range(1, len(WGRP))})

    def phase1(r, carry):
        x_copy(r).wait()
        wait_raw(r)

        @pl.when(r + 1 < NR1)
        def _():
            x_copy(r + 1).start()

        start_raw(jnp.minimum(r + 1, NR1))

        @pl.when(r == NR1 - 1)
        def _():
            woa_copy.start()

        wob_copy(r).start()
        r0 = pl.multiple_of(ROWS0 + r * ROWS1, ROWS1)
        qkv_dots(r0, ROWS1, chunk=r, never=jnp.full((8, 128), r, jnp.int32) < 0)
        return r

    with jax.named_scope('phase1'):
        lax.fori_loop(0, NR1, phase1, 0)

    S_ = (s0, s1)
    M_ = (m0, m1)
    QS = (qs0, qs1)
    qs0[...] = jnp.zeros_like(qs0)
    qs1[...] = jnp.zeros_like(qs1)

    def set_q(u, slot):
        g = u % G
        c0 = pl.multiple_of((u // G) * TQ, TQ)
        for h in range(4):
            QS[slot][h * 16:(h + 1) * 16, h * TQ:(h + 1) * TQ] = qt_s[g, h * 16:(h + 1) * 16, pl.ds(c0, TQ)]

    def scores_block(g, slot, kb, kw=None):
        kw = k_s[g, kb * (KB // 2):(kb + 1) * (KB // 2), :] if kw is None else kw
        sn = jnp.dot(_bf(kw), _bf(QS[slot][...]), preferred_element_type=F32)
        S_[slot][kb * KB:(kb + 1) * KB, :] = sn
        return sn.reshape(KB // 8, 8, 4 * TQ).max(axis=0)

    def finish_max(mrun, slot):
        M_[slot][...] = jnp.broadcast_to(jnp.max(mrun, axis=0, keepdims=True), (8, 4 * TQ))

    def a_slots(u, slot, never):
        un = jnp.minimum(u + 1, NU - 1)
        g = u % G
        cur, nxt = slot, 1 - slot
        set_q(un, nxt)
        m = M_[cur][...]
        mrun = None
        deps = {}
        l = [jnp.zeros((8, TQ), F32) for _ in range(4)]
        acc = [jnp.zeros((DHA, TQ), F32) for _ in range(4)]
        for kb in range(S // KB):
            mx = scores_block(un % G, nxt, kb)
            mrun = mx if mrun is None else jnp.maximum(mrun, mx)
            deps[kb] = mx
            for h in range(4):
                cols = slice(h * TQ, (h + 1) * TQ)
                mh = m[:, cols]
                if kb - 1 in deps:
                    mh = _after(never, deps[kb - 1][:, cols], mh)
                sc = S_[cur][kb * KB:(kb + 1) * KB, cols]
                p = jnp.exp2(sc.reshape(KB // 8, 8, TQ) - mh[None])
                l[h] = l[h] + p.sum(axis=0)
                vt = _bf(vt_s[g, h * 16:(h + 1) * 16, kb * KB:(kb + 1) * KB])
                acc[h] = acc[h] + jnp.dot(vt, p.reshape(KB, TQ).astype(BF16), preferred_element_type=F32)
            if kb < S // KB - 1:
                yield
        finish_max(mrun, nxt)
        ot = jnp.concatenate(
            [acc[h] / jnp.sum(l[h], axis=0, keepdims=True) for h in range(4)], axis=0)
        o_s[g] = _words(ot.T)
        yield

    scale_b = DHB ** -0.5
    qi = lax.broadcasted_iota(jnp.int32, (L, L), 0)
    ki = lax.broadcasted_iota(jnp.int32, (L, L), 1)
    mask = (qi < M) | (qi >= ki)

    def b_qkv(h):
        hx = h_s[...]
        bq_s[h] = jnp.dot(hx, _bf(wb_s[0, h]), preferred_element_type=F32)
        bk_s[h] = jnp.dot(hx, _bf(wb_s[1, h]), preferred_element_type=F32)
        bv_s[h] = jnp.dot(hx, _bf(wb_s[2, h]), preferred_element_type=F32)

    def b_scores(h):
        return lax.dot_general(bq_s[h], bk_s[h].astype(BF16), NT_DIMS, preferred_element_type=F32) * scale_b

    def b_softmax_pv(h, s_):
        s_ = jnp.where(mask, s_, -1000000000.0)
        m_ = jnp.max(s_, axis=-1, keepdims=True)
        p_ = jnp.exp(s_ - m_)
        l_ = jnp.sum(p_, axis=-1, keepdims=True)
        r_ = pltpu.reciprocal(l_, approx=True)
        r_ = r_ * (2.0 - l_ * r_)
        bo_s[:, h * DHB:(h + 1) * DHB] = jnp.dot(p_ * r_, bv_s[h].astype(BF16), preferred_element_type=F32)

    def fused_step(s, u0):
        never = jnp.full((8, TQ), s, jnp.int32) < 0
        a_iter = itertools.chain(a_slots(u0, 0, never), a_slots(u0 + 1, 1, never))
        AQ = 29
        TAIL = ("S", "A", "P", "A", "P", "A", "P")
        LS, LP = 1, 3
        n_a = 0
        r0 = pl.multiple_of(s * SEG, SEG)
        h_s[M:L, :] = xb_s[pl.ds(r0, SEG), :].astype(F32)
        sc, ns, npv = {}, 0, 0
        for t in range(HB):
            b_qkv(t)
            if (t + 1) * AQ // HB > t * AQ // HB:
                next(a_iter); n_a += 1
            if t >= LS:
                sc[ns] = b_scores(ns); ns += 1
            if t >= LP:
                b_softmax_pv(npv, sc.pop(npv)); npv += 1
        for tok in TAIL:
            if tok == "A":
                next(a_iter); n_a += 1
            elif tok == "S":
                sc[ns] = b_scores(ns); ns += 1
            else:
                b_softmax_pv(npv, sc.pop(npv)); npv += 1
        assert ns == HB and npv == HB
        rem = 32 - n_a
        mem = []
        for n in range(G):
            a = jnp.dot(bo_s[...], _bf(wob_w[n]), preferred_element_type=F32)
            out_s[pl.ds(r0, SEG), D + n * 128:D + (n + 1) * 128] = a[M:L].astype(BF16)
            mem.append(a[0:M])
            for _ in range((n + 1) * rem // G - n * rem // G):
                next(a_iter); n_a += 1
        assert n_a == 32
        h_s[0:M, :] = jnp.concatenate(mem, axis=1)

    set_q(0, 0)
    mrun = None
    for kb in range(S // KB):
        mx = scores_block(0, 0, kb)
        mrun = mx if mrun is None else jnp.maximum(mrun, mx)
    finish_max(mrun, 0)

    with jax.named_scope('restwait'):
        for c in [wob_copy(n) for n in range(G)] + [xb_first, mem0_copy, woa_copy]:
            c.wait()
        xb_rest.start()
    h_s[0:M, :] = mem0_s[...].astype(F32)

    def out_copy(j):
        rows = pl.ds(pl.multiple_of(j * TQ, TQ), TQ)
        return pltpu.make_async_copy(out_s.at[rows, :], out_hbm.at[rows, :], sem_out)

    def block(j, carry):
        @pl.when(j == 1)
        def _():
            xb_rest.wait()

        def inner(i, c):
            fused_step(j * SEG_PER_J + i, j * G + 2 * i)
            return c

        with jax.named_scope('inner'):
            lax.fori_loop(0, SEG_PER_J, inner, 0)

        r0 = pl.multiple_of(j * TQ, TQ)
        ob = jnp.concatenate([_bf(o_s[g]) for g in range(G)], axis=1)
        for n in range(G):
            y = jnp.dot(ob, woa_s[:, n * 128:(n + 1) * 128], preferred_element_type=F32)
            out_s[pl.ds(r0, TQ), n * 128:(n + 1) * 128] = y.astype(BF16)
        out_copy(j).start()
        return carry

    with jax.named_scope('main'):
        lax.fori_loop(0, NJ, block, 0)
    for j in range(NJ):
        out_copy(j).wait()


@functools.partial(jax.jit, static_argnames=("B_seg_len",))
def pallas_concat_heads__softmax_full_mha__memory_aug_recurrent_mem_tr__prompt_kernel(
    A_x: jax.Array,
    A_wqkv: jax.Array,
    A_wo: jax.Array,
    B_x: jax.Array,
    B_mem0: jax.Array,
    B_Wq: jax.Array,
    B_Wk: jax.Array,
    B_Wv: jax.Array,
    B_Wo: jax.Array,
    B_seg_len: int,
):
    _, S, D = A_x.shape
    _, HB, DHB = B_Wq.shape
    M = B_mem0.shape[1]
    SEG = int(B_seg_len)
    L = M + SEG
    G = D // 128
    assert 4 * SEG == TQ and G == 2 * (TQ // SEG)

    vm = pltpu.VMEM
    scratch = [
        vm((S, D), BF16),
        vm((D, 3 * D), BF16),
        vm((D, D), BF16),
        vm((S, D), BF16),
        vm((M, D), BF16),
        vm((G, HB * DHB, 128), BF16),
        vm((2, D // 2, HB, DHB), BF16),
        vm((3, HB, D // 2, DHB), U32),
        vm((G, 64, S), U32),
        vm((G, S // 2, 128), U32),
        vm((G, 64, S), U32),
        vm((S, 4 * TQ), F32),
        vm((S, 4 * TQ), F32),
        vm((8, 4 * TQ), F32),
        vm((8, 4 * TQ), F32),
        vm((64, 4 * TQ), U32),
        vm((64, 4 * TQ), U32),
        vm((G, TQ // 2, 128), U32),
        vm((L, D), F32),
        vm((HB, L, DHB), F32),
        vm((HB, L, DHB), F32),
        vm((HB, L, DHB), F32),
        vm((L, HB * DHB), F32),
        vm((S, 2 * D), BF16),
        pltpu.SemaphoreType.DMA((8,)),
        pltpu.SemaphoreType.DMA((5,)),
        pltpu.SemaphoreType.DMA((2,)),
        pltpu.SemaphoreType.DMA,
        pltpu.SemaphoreType.DMA,
        pltpu.SemaphoreType.DMA,
        pltpu.SemaphoreType.DMA,
    ]
    any_spec = pl.BlockSpec(memory_space=pl.ANY)
    out = pl.pallas_call(
        functools.partial(_kernel, S=S, D=D, HB=HB, DHB=DHB, M=M, SEG=SEG),
        out_shape=jax.ShapeDtypeStruct((S, 2 * D), A_x.dtype),
        in_specs=[any_spec] * 9,
        out_specs=any_spec,
        scratch_shapes=scratch,
        compiler_params=pltpu.CompilerParams(vmem_limit_bytes=120 * 1024 * 1024),
        name="fused_mha_rmt",
    )(
        A_x.reshape(S, D), A_wqkv, A_wo, B_x.reshape(S, D), B_mem0.reshape(M, D),
        B_Wq, B_Wk, B_Wv, B_Wo.reshape(HB * DHB, D),
    )
    return out.reshape(1, S, 2 * D)
```

```python
import functools
import itertools

import jax
import jax.numpy as jnp
from jax import lax
import jax.experimental.pallas as pl
import jax.experimental.pallas.tpu as pltpu

F32 = jnp.float32
BF16 = jnp.bfloat16
U32 = jnp.uint32
LOG2E = 1.4426950408889634
NT_DIMS = (((1,), (1,)), ((), ()))

A_HEADS = 32
TQ = 128
KB = 128
ROWS0 = 512
ROWS1 = 256


def _bf(words):
    return pltpu.bitcast(words, BF16)


def _words(x_f32):
    return pltpu.bitcast(x_f32.astype(BF16), U32)


def _after(never, dep, val):
    return jnp.where(never, dep, val)


def _kernel(
    xa_hbm, wqkv_hbm, woa_hbm, xb_hbm, mem0_hbm, wq_hbm, wk_hbm, wv_hbm, wob_hbm,
    out_hbm,
    xa_s, wqkv_s, woa_s, xb_s, mem0_s, wob_s, raw_s, wb_s,
    qt_s, k_s, vt_s, s0, s1, m0, m1, qs0, qs1, o_s,
    h_s, bq_s, bk_s, bv_s, bo_s, out_s,
    sem_x, sem_w, sem_raw, sem_early, sem_xb, sem_woa, sem_out,
    *, S, D, HB, DHB, M, SEG,
):
    G = D // 128
    DHA = D // A_HEADS
    NJ = S // TQ
    NU = G * NJ
    L = M + SEG
    NR1 = (S - ROWS0) // ROWS1
    DCH = D // 2
    assert NR1 == 6
    SEG_PER_J = TQ // SEG

    x_first = pltpu.make_async_copy(xa_hbm.at[pl.ds(0, ROWS0), :], xa_s.at[pl.ds(0, ROWS0), :], sem_x.at[NR1])

    def x_copy(r):
        rows = pl.ds(ROWS0 + r * ROWS1, ROWS1)
        return pltpu.make_async_copy(xa_hbm.at[rows, :], xa_s.at[rows, :], sem_x.at[r])

    WGRP = [(0, 2), (2, 6), (6, 14), (14, 24)]

    def wqkv_copies(grp):
        lo, hi = WGRP[grp]
        out = []
        n = lo
        while n < hi:
            e = min(hi, (n // G + 1) * G)
            c0 = ((0, 2, 1)[n // G] * G + n % G) * 128
            cols = pl.ds(c0, (e - n) * 128)
            out.append(pltpu.make_async_copy(wqkv_hbm.at[:, cols], wqkv_s.at[:, cols], sem_w.at[grp]))
            n = e
        return out

    def raw_copy(i, half, slot):
        w = (wq_hbm, wk_hbm, wv_hbm)[i]
        return pltpu.make_async_copy(w.at[pl.ds(half * DCH, DCH)], raw_s.at[slot], sem_raw.at[slot])

    def start_raw(c):
        for i in range(3):
            @pl.when(c // 2 == i)
            def _():
                raw_copy(i, c % 2, c % 2).start()

    def wait_raw(c):
        raw_copy(0, 0, c % 2).wait()

    def wob_copy(n):
        return pltpu.make_async_copy(wob_hbm.at[:, pl.ds(n * 128, 128)], wob_s.at[n], sem_early)

    xb_first = pltpu.make_async_copy(xb_hbm.at[pl.ds(0, TQ), :], xb_s.at[pl.ds(0, TQ), :], sem_early)
    xb_rest = pltpu.make_async_copy(xb_hbm.at[pl.ds(TQ, S - TQ), :], xb_s.at[pl.ds(TQ, S - TQ), :], sem_xb)
    mem0_copy = pltpu.make_async_copy(mem0_hbm, mem0_s, sem_early)
    woa_copy = pltpu.make_async_copy(woa_hbm, woa_s, sem_woa)

    wob_w = wob_s.bitcast(U32)

    q_mul = (DHA ** -0.5) * LOG2E
    sub8 = lax.broadcasted_iota(jnp.int32, (8, 128), 0)
    PART_ORDER = (0, 2, 1)
    pieces = [(dd, half) for dd in range(0, DCH, 16) for half in range(HB // 16)]

    def relayout_piece(c, dd, half, gate=None, never=None):
        slot = c % 2
        rows = pl.ds(pl.multiple_of(slot * (DCH // 2) + dd // 2, 8), 8)
        wsel = c // 2
        ev, od = [], []
        for t in range(8):
            a = pltpu.bitcast(raw_s[slot, dd + 2 * t, half * 16:(half + 1) * 16, :], U32)
            b = pltpu.bitcast(raw_s[slot, dd + 2 * t + 1, half * 16:(half + 1) * 16, :], U32)
            if gate is not None:
                a = _after(never, gate, a)
            ev.append((a & U32(0xFFFF)) | (b << 16))
            od.append((a >> 16) | (b & U32(0xFFFF0000)))
        for par, v in ((0, ev), (1, od)):
            for k in (1, 2, 4):
                msk = (sub8 & k) == 0
                nv = list(v)
                for t in range(8):
                    if t & k == 0:
                        x_, y_ = v[t], v[t + k]
                        nv[t] = jnp.where(msk, x_, pltpu.roll(y_, k, 0))
                        nv[t + k] = jnp.where(msk, pltpu.roll(x_, 8 - k, 0), y_)
                v = nv
            for t in range(8):
                wb_s[wsel, 2 * (half * 8 + t) + par, rows, :] = v[t]
        return wb_s[wsel, half * 16 + 15, rows, :]

    def qkv_dots(r0, rows, chunk=None, never=None, hooks=None):
        xt = xa_s[pl.ds(r0, rows), :]
        deps = {}
        gate = None
        npc = len(pieces)
        LAG, GSTEP = 2, 80
        NPS = 3 * G - 2
        for n in range(3 * G):
            if hooks and n in hooks:
                hooks[n]()
            part, g = PART_ORDER[n // G], n % G
            col = part * G + g
            w = wqkv_s[:, col * 128:(col + 1) * 128]
            if n - LAG in deps:
                w = jnp.concatenate([_bf(_after(never, deps[n - LAG], pltpu.bitcast(w[0:16], U32))), w[16:]], axis=0)
            y = jnp.dot(xt, w, preferred_element_type=F32)
            if chunk is not None:
                lo, hi = min(n, NPS) * npc // NPS, min(n + 1, NPS) * npc // NPS
                for t in range(lo, hi):
                    gt = None if gate is None else gate[(t - lo) * GSTEP:(t - lo) * GSTEP + 8]
                    deps[n] = relayout_piece(chunk, *pieces[t], gate=gt, never=never)
            gate = pltpu.bitcast(y, U32)
            if part == 0:
                qt_s[g, :, pl.ds(r0, rows)] = _words((y * q_mul).T)
            elif part == 1:
                k_s[g, pl.ds(pl.multiple_of(r0 // 2, rows // 2), rows // 2), :] = _words(y)
            else:
                vt_s[g, :, pl.ds(r0, rows)] = _words(y.T)

    with jax.named_scope('first'):
        def start(grp):
            for c in wqkv_copies(grp):
                c.start()

        def wait(grp):
            for c in wqkv_copies(grp):
                c.wait()

        x_first.start()
        start(0)
        x_first.wait()
        wait(0)
        start(1)
        start(2)

        def hook(k):
            def run():
                wait(k)
                if k + 2 < len(WGRP):
                    start(k + 2)
                elif k + 2 == len(WGRP):
                    raw_copy(0, 0, 0).start()
                else:
                    for c in [x_copy(0), wob_copy(6), wob_copy(7), xb_first, mem0_copy]:
                        c.start()
            return run

        qkv_dots(0, ROWS0, hooks={WGRP[k][0]: hook(k) for k in range(1, len(WGRP))})

    def phase1(r, carry):
        x_copy(r).wait()
        wait_raw(r)

        @pl.when(r + 1 < NR1)
        def _():
            x_copy(r + 1).start()

        start_raw(jnp.minimum(r + 1, NR1))

        @pl.when(r == NR1 - 1)
        def _():
            woa_copy.start()

        wob_copy(r).start()
        r0 = pl.multiple_of(ROWS0 + r * ROWS1, ROWS1)
        qkv_dots(r0, ROWS1, chunk=r, never=jnp.full((8, 128), r, jnp.int32) < 0)
        return r

    with jax.named_scope('phase1'):
        lax.fori_loop(0, NR1, phase1, 0)

    S_ = (s0, s1)
    M_ = (m0, m1)
    QS = (qs0, qs1)
    qs0[...] = jnp.zeros_like(qs0)
    qs1[...] = jnp.zeros_like(qs1)

    def set_q(u, slot):
        g = u % G
        c0 = pl.multiple_of((u // G) * TQ, TQ)
        for h in range(4):
            QS[slot][h * 16:(h + 1) * 16, h * TQ:(h + 1) * TQ] = qt_s[g, h * 16:(h + 1) * 16, pl.ds(c0, TQ)]

    def scores_block(g, slot, kb, kw=None):
        kw = k_s[g, kb * (KB // 2):(kb + 1) * (KB // 2), :] if kw is None else kw
        sn = jnp.dot(_bf(kw), _bf(QS[slot][...]), preferred_element_type=F32)
        S_[slot][kb * KB:(kb + 1) * KB, :] = sn
        return sn.reshape(KB // 8, 8, 4 * TQ).max(axis=0)

    def finish_max(mrun, slot):
        M_[slot][...] = jnp.broadcast_to(jnp.max(mrun, axis=0, keepdims=True), (8, 4 * TQ))

    def a_slots(u, slot, never):
        un = jnp.minimum(u + 1, NU - 1)
        g = u % G
        cur, nxt = slot, 1 - slot
        set_q(un, nxt)
        m = M_[cur][...]
        mrun = None
        deps = {}
        l = [jnp.zeros((8, TQ), F32) for _ in range(4)]
        acc = [jnp.zeros((DHA, TQ), F32) for _ in range(4)]
        for kb in range(S // KB):
            mx = scores_block(un % G, nxt, kb)
            mrun = mx if mrun is None else jnp.maximum(mrun, mx)
            deps[kb] = mx
            for h in range(4):
                cols = slice(h * TQ, (h + 1) * TQ)
                mh = m[:, cols]
                if kb - 1 in deps:
                    mh = _after(never, deps[kb - 1][:, cols], mh)
                sc = S_[cur][kb * KB:(kb + 1) * KB, cols]
                p = jnp.exp2(sc.reshape(KB // 8, 8, TQ) - mh[None])
                l[h] = l[h] + p.sum(axis=0)
                vt = _bf(vt_s[g, h * 16:(h + 1) * 16, kb * KB:(kb + 1) * KB])
                acc[h] = acc[h] + jnp.dot(vt, p.reshape(KB, TQ).astype(BF16), preferred_element_type=F32)
            if kb < S // KB - 1:
                yield
        finish_max(mrun, nxt)
        ot = jnp.concatenate(
            [acc[h] / jnp.sum(l[h], axis=0, keepdims=True) for h in range(4)], axis=0)
        o_s[g] = _words(ot.T)
        yield

    scale_b = DHB ** -0.5
    qi = lax.broadcasted_iota(jnp.int32, (L, L), 0)
    ki = lax.broadcasted_iota(jnp.int32, (L, L), 1)
    mask = (qi < M) | (qi >= ki)

    def b_qkv(h):
        hx = h_s[...]
        bq_s[h] = jnp.dot(hx, _bf(wb_s[0, h]), preferred_element_type=F32)
        bk_s[h] = jnp.dot(hx, _bf(wb_s[1, h]), preferred_element_type=F32)
        bv_s[h] = jnp.dot(hx, _bf(wb_s[2, h]), preferred_element_type=F32)

    def b_scores(h):
        return lax.dot_general(bq_s[h], bk_s[h].astype(BF16), NT_DIMS, preferred_element_type=F32) * scale_b

    def b_softmax_pv(h, s_):
        s_ = jnp.where(mask, s_, -1000000000.0)
        m_ = jnp.max(s_, axis=-1, keepdims=True)
        p_ = jnp.exp(s_ - m_)
        l_ = jnp.sum(p_, axis=-1, keepdims=True)
        r_ = pltpu.reciprocal(l_, approx=True)
        r_ = r_ * (2.0 - l_ * r_)
        bo_s[:, h * DHB:(h + 1) * DHB] = jnp.dot(p_ * r_, bv_s[h].astype(BF16), preferred_element_type=F32)

    def fused_step(s, u0):
        never = jnp.full((8, TQ), s, jnp.int32) < 0
        a_iter = itertools.chain(a_slots(u0, 0, never), a_slots(u0 + 1, 1, never))
        AQ = 29
        TAIL = ("S", "A", "P", "A", "P", "A", "P")
        LS, LP = 1, 3
        n_a = 0
        r0 = pl.multiple_of(s * SEG, SEG)
        h_s[M:L, :] = xb_s[pl.ds(r0, SEG), :].astype(F32)
        sc, ns, npv = {}, 0, 0
        for t in range(HB):
            b_qkv(t)
            if (t + 1) * AQ // HB > t * AQ // HB:
                next(a_iter); n_a += 1
            if t >= LS:
                sc[ns] = b_scores(ns); ns += 1
            if t >= LP:
                b_softmax_pv(npv, sc.pop(npv)); npv += 1
        for tok in TAIL:
            if tok == "A":
                next(a_iter); n_a += 1
            elif tok == "S":
                sc[ns] = b_scores(ns); ns += 1
            else:
                b_softmax_pv(npv, sc.pop(npv)); npv += 1
        assert ns == HB and npv == HB
        rem = 32 - n_a
        mem = []
        for n in range(G):
            a = jnp.dot(bo_s[...], _bf(wob_w[n]), preferred_element_type=F32)
            out_s[pl.ds(r0, SEG), D + n * 128:D + (n + 1) * 128] = a[M:L].astype(BF16)
            mem.append(a[0:M])
            for _ in range((n + 1) * rem // G - n * rem // G):
                next(a_iter); n_a += 1
        assert n_a == 32
        h_s[0:M, :] = jnp.concatenate(mem, axis=1)

    set_q(0, 0)
    mrun = None
    for kb in range(S // KB):
        mx = scores_block(0, 0, kb)
        mrun = mx if mrun is None else jnp.maximum(mrun, mx)
    finish_max(mrun, 0)

    with jax.named_scope('restwait'):
        for c in [wob_copy(n) for n in range(G)] + [xb_first, mem0_copy, woa_copy]:
            c.wait()
        xb_rest.start()
    h_s[0:M, :] = mem0_s[...].astype(F32)

    def out_copy(j):
        rows = pl.ds(pl.multiple_of(j * TQ, TQ), TQ)
        return pltpu.make_async_copy(out_s.at[rows, :], out_hbm.at[rows, :], sem_out)

    def block(j, carry):
        @pl.when(j == 1)
        def _():
            xb_rest.wait()

        def inner(i, c):
            fused_step(j * SEG_PER_J + i, j * G + 2 * i)
            return c

        with jax.named_scope('inner'):
            lax.fori_loop(0, SEG_PER_J, inner, 0)

        r0 = pl.multiple_of(j * TQ, TQ)
        ob = jnp.concatenate([_bf(o_s[g]) for g in range(G)], axis=1)
        for n in range(G):
            y = jnp.dot(ob, woa_s[:, n * 128:(n + 1) * 128], preferred_element_type=F32)
            out_s[pl.ds(r0, TQ), n * 128:(n + 1) * 128] = y.astype(BF16)
        out_copy(j).start()
        return carry

    with jax.named_scope('main'):
        lax.fori_loop(0, NJ, block, 0)
    for j in range(NJ):
        out_copy(j).wait()


@functools.partial(jax.jit, static_argnames=("B_seg_len",))
def pallas_concat_heads__softmax_full_mha__memory_aug_recurrent_mem_tr__prompt_kernel(
    A_x: jax.Array,
    A_wqkv: jax.Array,
    A_wo: jax.Array,
    B_x: jax.Array,
    B_mem0: jax.Array,
    B_Wq: jax.Array,
    B_Wk: jax.Array,
    B_Wv: jax.Array,
    B_Wo: jax.Array,
    B_seg_len: int,
):
    _, S, D = A_x.shape
    _, HB, DHB = B_Wq.shape
    M = B_mem0.shape[1]
    SEG = int(B_seg_len)
    L = M + SEG
    G = D // 128
    assert 4 * SEG == TQ and G == 2 * (TQ // SEG)

    vm = pltpu.VMEM
    scratch = [
        vm((S, D), BF16),
        vm((D, 3 * D), BF16),
        vm((D, D), BF16),
        vm((S, D), BF16),
        vm((M, D), BF16),
        vm((G, HB * DHB, 128), BF16),
        vm((2, D // 2, HB, DHB), BF16),
        vm((3, HB, D // 2, DHB), U32),
        vm((G, 64, S), U32),
        vm((G, S // 2, 128), U32),
        vm((G, 64, S), U32),
        vm((S, 4 * TQ), F32),
        vm((S, 4 * TQ), F32),
        vm((8, 4 * TQ), F32),
        vm((8, 4 * TQ), F32),
        vm((64, 4 * TQ), U32),
        vm((64, 4 * TQ), U32),
        vm((G, TQ // 2, 128), U32),
        vm((L, D), F32),
        vm((HB, L, DHB), F32),
        vm((HB, L, DHB), F32),
        vm((HB, L, DHB), F32),
        vm((L, HB * DHB), F32),
        vm((S, 2 * D), BF16),
        pltpu.SemaphoreType.DMA((8,)),
        pltpu.SemaphoreType.DMA((5,)),
        pltpu.SemaphoreType.DMA((2,)),
        pltpu.SemaphoreType.DMA,
        pltpu.SemaphoreType.DMA,
        pltpu.SemaphoreType.DMA,
        pltpu.SemaphoreType.DMA,
    ]
    any_spec = pl.BlockSpec(memory_space=pl.ANY)
    out = pl.pallas_call(
        functools.partial(_kernel, S=S, D=D, HB=HB, DHB=DHB, M=M, SEG=SEG),
        out_shape=jax.ShapeDtypeStruct((S, 2 * D), A_x.dtype),
        in_specs=[any_spec] * 9,
        out_specs=any_spec,
        scratch_shapes=scratch,
        compiler_params=pltpu.CompilerParams(vmem_limit_bytes=120 * 1024 * 1024),
        name="fused_mha_rmt",
    )(
        A_x.reshape(S, D), A_wqkv, A_wo, B_x.reshape(S, D), B_mem0.reshape(M, D),
        B_Wq, B_Wk, B_Wv, B_Wo.reshape(HB * DHB, D),
    )
    return out.reshape(1, S, 2 * D)
```

```python
import functools
import itertools

import jax
import jax.numpy as jnp
from jax import lax
import jax.experimental.pallas as pl
import jax.experimental.pallas.tpu as pltpu

F32 = jnp.float32
BF16 = jnp.bfloat16
U32 = jnp.uint32
LOG2E = 1.4426950408889634
NT_DIMS = (((1,), (1,)), ((), ()))

A_HEADS = 32
TQ = 128
KB = 128
ROWS0 = 512
ROWS1 = 256


def _bf(words):
    return pltpu.bitcast(words, BF16)


def _words(x_f32):
    return pltpu.bitcast(x_f32.astype(BF16), U32)


def _after(never, dep, val):
    return jnp.where(never, dep, val)


def _kernel(
    xa_hbm, wqkv_hbm, woa_hbm, xb_hbm, mem0_hbm, wq_hbm, wk_hbm, wv_hbm, wob_hbm,
    out_hbm,
    xa_s, wqkv_s, woa_s, xb_s, mem0_s, wob_s, raw_s, wb_s,
    qt_s, k_s, vt_s, s0, s1, m0, m1, qs0, qs1, o_s,
    h_s, bq_s, bk_s, bv_s, bo_s, out_s,
    sem_x, sem_w, sem_raw, sem_early, sem_xb, sem_woa, sem_out,
    *, S, D, HB, DHB, M, SEG,
):
    G = D // 128
    DHA = D // A_HEADS
    NJ = S // TQ
    NU = G * NJ
    L = M + SEG
    NR1 = (S - ROWS0) // ROWS1
    DCH = D // 2
    assert NR1 == 6
    SEG_PER_J = TQ // SEG

    x_first = pltpu.make_async_copy(xa_hbm.at[pl.ds(0, ROWS0), :], xa_s.at[pl.ds(0, ROWS0), :], sem_x.at[NR1])

    def x_copy(r):
        rows = pl.ds(ROWS0 + r * ROWS1, ROWS1)
        return pltpu.make_async_copy(xa_hbm.at[rows, :], xa_s.at[rows, :], sem_x.at[r])

    WGRP = [(0, 2), (2, 6), (6, 14), (14, 24)]

    def wqkv_copies(grp):
        lo, hi = WGRP[grp]
        out = []
        n = lo
        while n < hi:
            e = min(hi, (n // G + 1) * G)
            c0 = ((0, 2, 1)[n // G] * G + n % G) * 128
            cols = pl.ds(c0, (e - n) * 128)
            out.append(pltpu.make_async_copy(wqkv_hbm.at[:, cols], wqkv_s.at[:, cols], sem_w.at[grp]))
            n = e
        return out

    def raw_copy(i, half, slot):
        w = (wq_hbm, wk_hbm, wv_hbm)[i]
        return pltpu.make_async_copy(w.at[pl.ds(half * DCH, DCH)], raw_s.at[slot], sem_raw.at[slot])

    def start_raw(c):
        for i in range(3):
            @pl.when(c // 2 == i)
            def _():
                raw_copy(i, c % 2, c % 2).start()

    def wait_raw(c):
        raw_copy(0, 0, c % 2).wait()

    def wob_copy(n):
        return pltpu.make_async_copy(wob_hbm.at[:, pl.ds(n * 128, 128)], wob_s.at[n], sem_early)

    xb_first = pltpu.make_async_copy(xb_hbm.at[pl.ds(0, TQ), :], xb_s.at[pl.ds(0, TQ), :], sem_early)
    xb_rest = pltpu.make_async_copy(xb_hbm.at[pl.ds(TQ, S - TQ), :], xb_s.at[pl.ds(TQ, S - TQ), :], sem_xb)
    mem0_copy = pltpu.make_async_copy(mem0_hbm, mem0_s, sem_early)
    woa_copy = pltpu.make_async_copy(woa_hbm, woa_s, sem_woa)

    wob_w = wob_s.bitcast(U32)

    q_mul = (DHA ** -0.5) * LOG2E
    sub8 = lax.broadcasted_iota(jnp.int32, (8, 128), 0)
    PART_ORDER = (0, 2, 1)
    pieces = [(dd, half) for dd in range(0, DCH, 16) for half in range(HB // 16)]

    def relayout_piece(c, dd, half, gate=None, never=None):
        slot = c % 2
        rows = pl.ds(pl.multiple_of(slot * (DCH // 2) + dd // 2, 8), 8)
        wsel = c // 2
        ev, od = [], []
        for t in range(8):
            a = pltpu.bitcast(raw_s[slot, dd + 2 * t, half * 16:(half + 1) * 16, :], U32)
            b = pltpu.bitcast(raw_s[slot, dd + 2 * t + 1, half * 16:(half + 1) * 16, :], U32)
            if gate is not None:
                a = _after(never, gate, a)
            ev.append((a & U32(0xFFFF)) | (b << 16))
            od.append((a >> 16) | (b & U32(0xFFFF0000)))
        for par, v in ((0, ev), (1, od)):
            for k in (1, 2, 4):
                msk = (sub8 & k) == 0
                nv = list(v)
                for t in range(8):
                    if t & k == 0:
                        x_, y_ = v[t], v[t + k]
                        nv[t] = jnp.where(msk, x_, pltpu.roll(y_, k, 0))
                        nv[t + k] = jnp.where(msk, pltpu.roll(x_, 8 - k, 0), y_)
                v = nv
            for t in range(8):
                wb_s[wsel, 2 * (half * 8 + t) + par, rows, :] = v[t]
        return wb_s[wsel, half * 16 + 15, rows, :]

    def qkv_dots(r0, rows, chunk=None, never=None, hooks=None):
        xt = xa_s[pl.ds(r0, rows), :]
        deps = {}
        gate = None
        npc = len(pieces)
        LAG, GSTEP = 2, 80
        NPS = 3 * G - 2
        for n in range(3 * G):
            if hooks and n in hooks:
                hooks[n]()
            part, g = PART_ORDER[n // G], n % G
            col = part * G + g
            w = wqkv_s[:, col * 128:(col + 1) * 128]
            if n - LAG in deps:
                w = jnp.concatenate([_bf(_after(never, deps[n - LAG], pltpu.bitcast(w[0:16], U32))), w[16:]], axis=0)
            y = jnp.dot(xt, w, preferred_element_type=F32)
            if chunk is not None:
                lo, hi = min(n, NPS) * npc // NPS, min(n + 1, NPS) * npc // NPS
                for t in range(lo, hi):
                    gt = None if gate is None else gate[(t - lo) * GSTEP:(t - lo) * GSTEP + 8]
                    deps[n] = relayout_piece(chunk, *pieces[t], gate=gt, never=never)
            gate = pltpu.bitcast(y, U32)
            if part == 0:
                qt_s[g, :, pl.ds(r0, rows)] = _words((y * q_mul).T)
            elif part == 1:
                k_s[g, pl.ds(pl.multiple_of(r0 // 2, rows // 2), rows // 2), :] = _words(y)
            else:
                vt_s[g, :, pl.ds(r0, rows)] = _words(y.T)

    with jax.named_scope('first'):
        def start(grp):
            for c in wqkv_copies(grp):
                c.start()

        def wait(grp):
            for c in wqkv_copies(grp):
                c.wait()

        x_first.start()
        start(0)
        qs0[...] = jnp.zeros_like(qs0)
        qs1[...] = jnp.zeros_like(qs1)
        x_first.wait()
        wait(0)
        start(1)
        start(2)

        def hook(k):
            def run():
                wait(k)
                if k + 2 < len(WGRP):
                    start(k + 2)
                elif k + 2 == len(WGRP):
                    raw_copy(0, 0, 0).start()
                else:
                    for c in [x_copy(0), wob_copy(6), wob_copy(7), xb_first, mem0_copy]:
                        c.start()
            return run

        qkv_dots(0, ROWS0, hooks={WGRP[k][0]: hook(k) for k in range(1, len(WGRP))})

    def phase1(r, carry):
        wob_copy(r).start()
        x_copy(r).wait()
        wait_raw(r)

        @pl.when(r + 1 < NR1)
        def _():
            x_copy(r + 1).start()

        start_raw(jnp.minimum(r + 1, NR1))

        @pl.when(r == NR1 - 1)
        def _():
            woa_copy.start()

        r0 = pl.multiple_of(ROWS0 + r * ROWS1, ROWS1)
        qkv_dots(r0, ROWS1, chunk=r, never=jnp.full((8, 128), r, jnp.int32) < 0)
        return r

    with jax.named_scope('phase1'):
        lax.fori_loop(0, NR1, phase1, 0)

    S_ = (s0, s1)
    M_ = (m0, m1)
    QS = (qs0, qs1)

    def set_q(u, slot):
        g = u % G
        c0 = pl.multiple_of((u // G) * TQ, TQ)
        for h in range(4):
            QS[slot][h * 16:(h + 1) * 16, h * TQ:(h + 1) * TQ] = qt_s[g, h * 16:(h + 1) * 16, pl.ds(c0, TQ)]

    def scores_block(g, slot, kb, kw=None):
        kw = k_s[g, kb * (KB // 2):(kb + 1) * (KB // 2), :] if kw is None else kw
        sn = jnp.dot(_bf(kw), _bf(QS[slot][...]), preferred_element_type=F32)
        S_[slot][kb * KB:(kb + 1) * KB, :] = sn
        return sn.reshape(KB // 8, 8, 4 * TQ).max(axis=0)

    def finish_max(mrun, slot):
        M_[slot][...] = jnp.broadcast_to(jnp.max(mrun, axis=0, keepdims=True), (8, 4 * TQ))

    def a_slots(u, slot, never):
        un = jnp.minimum(u + 1, NU - 1)
        g = u % G
        cur, nxt = slot, 1 - slot
        set_q(un, nxt)
        m = M_[cur][...]
        mrun = None
        deps = {}
        l = [jnp.zeros((8, TQ), F32) for _ in range(4)]
        acc = [jnp.zeros((DHA, TQ), F32) for _ in range(4)]
        for kb in range(S // KB):
            mx = scores_block(un % G, nxt, kb)
            mrun = mx if mrun is None else jnp.maximum(mrun, mx)
            deps[kb] = mx
            for h in range(4):
                cols = slice(h * TQ, (h + 1) * TQ)
                mh = m[:, cols]
                if kb - 1 in deps:
                    mh = _after(never, deps[kb - 1][:, cols], mh)
                sc = S_[cur][kb * KB:(kb + 1) * KB, cols]
                p = jnp.exp2(sc.reshape(KB // 8, 8, TQ) - mh[None])
                l[h] = l[h] + p.sum(axis=0)
                vt = _bf(vt_s[g, h * 16:(h + 1) * 16, kb * KB:(kb + 1) * KB])
                acc[h] = acc[h] + jnp.dot(vt, p.reshape(KB, TQ).astype(BF16), preferred_element_type=F32)
            if kb < S // KB - 1:
                yield
        finish_max(mrun, nxt)
        ot = jnp.concatenate(
            [acc[h] / jnp.sum(l[h], axis=0, keepdims=True) for h in range(4)], axis=0)
        o_s[g] = _words(ot.T)
        yield

    scale_b = DHB ** -0.5
    qi = lax.broadcasted_iota(jnp.int32, (L, L), 0)
    ki = lax.broadcasted_iota(jnp.int32, (L, L), 1)
    mask = (qi < M) | (qi >= ki)

    def b_qkv(h):
        hx = h_s[...]
        bq_s[h] = jnp.dot(hx, _bf(wb_s[0, h]), preferred_element_type=F32)
        bk_s[h] = jnp.dot(hx, _bf(wb_s[1, h]), preferred_element_type=F32)
        bv_s[h] = jnp.dot(hx, _bf(wb_s[2, h]), preferred_element_type=F32)

    def b_scores(h):
        return lax.dot_general(bq_s[h], bk_s[h].astype(BF16), NT_DIMS, preferred_element_type=F32) * scale_b

    def b_softmax_pv(h, s_):
        s_ = jnp.where(mask, s_, -1000000000.0)
        m_ = jnp.max(s_, axis=-1, keepdims=True)
        p_ = jnp.exp(s_ - m_)
        l_ = jnp.sum(p_, axis=-1, keepdims=True)
        r_ = pltpu.reciprocal(l_, approx=True)
        r_ = r_ * (2.0 - l_ * r_)
        bo_s[:, h * DHB:(h + 1) * DHB] = jnp.dot(p_ * r_, bv_s[h].astype(BF16), preferred_element_type=F32)

    def fused_step(s, u0):
        never = jnp.full((8, TQ), s, jnp.int32) < 0
        a_iter = itertools.chain(a_slots(u0, 0, never), a_slots(u0 + 1, 1, never))
        AQ = 29
        TAIL = ("S", "A", "P", "A", "P", "A", "P")
        LS, LP = 1, 3
        n_a = 0
        r0 = pl.multiple_of(s * SEG, SEG)
        h_s[M:L, :] = xb_s[pl.ds(r0, SEG), :].astype(F32)
        sc, ns, npv = {}, 0, 0
        for t in range(HB):
            b_qkv(t)
            if (t + 1) * AQ // HB > t * AQ // HB:
                next(a_iter); n_a += 1
            if t >= LS:
                sc[ns] = b_scores(ns); ns += 1
            if t >= LP:
                b_softmax_pv(npv, sc.pop(npv)); npv += 1
        for tok in TAIL:
            if tok == "A":
                next(a_iter); n_a += 1
            elif tok == "S":
                sc[ns] = b_scores(ns); ns += 1
            else:
                b_softmax_pv(npv, sc.pop(npv)); npv += 1
        assert ns == HB and npv == HB
        rem = 32 - n_a
        mem = []
        for n in range(G):
            a = jnp.dot(bo_s[...], _bf(wob_w[n]), preferred_element_type=F32)
            out_s[pl.ds(r0, SEG), D + n * 128:D + (n + 1) * 128] = a[M:L].astype(BF16)
            mem.append(a[0:M])
            for _ in range((n + 1) * rem // G - n * rem // G):
                next(a_iter); n_a += 1
        assert n_a == 32
        h_s[0:M, :] = jnp.concatenate(mem, axis=1)

    set_q(0, 0)
    mrun = None
    for kb in range(S // KB):
        mx = scores_block(0, 0, kb)
        mrun = mx if mrun is None else jnp.maximum(mrun, mx)
    finish_max(mrun, 0)

    with jax.named_scope('restwait'):
        for c in [wob_copy(n) for n in range(G)] + [xb_first, mem0_copy, woa_copy]:
            c.wait()
        xb_rest.start()
    h_s[0:M, :] = mem0_s[...].astype(F32)

    def out_copy(j, half):
        rows = pl.ds(pl.multiple_of(j * TQ, TQ), TQ)
        cols = pl.ds(half * D, D)
        return pltpu.make_async_copy(out_s.at[rows, cols], out_hbm.at[rows, cols], sem_out)

    def block(j, carry):
        @pl.when(j == 1)
        def _():
            xb_rest.wait()

        def inner(i, c):
            fused_step(j * SEG_PER_J + i, j * G + 2 * i)
            return c

        with jax.named_scope('inner'):
            lax.fori_loop(0, SEG_PER_J, inner, 0)
        out_copy(j, 1).start()

        r0 = pl.multiple_of(j * TQ, TQ)
        ob = jnp.concatenate([_bf(o_s[g]) for g in range(G)], axis=1)
        for n in range(G):
            y = jnp.dot(ob, woa_s[:, n * 128:(n + 1) * 128], preferred_element_type=F32)
            out_s[pl.ds(r0, TQ), n * 128:(n + 1) * 128] = y.astype(BF16)
        out_copy(j, 0).start()
        return carry

    with jax.named_scope('main'):
        lax.fori_loop(0, NJ, block, 0)
    for j in range(NJ):
        out_copy(j, 0).wait()
        out_copy(j, 1).wait()


@functools.partial(jax.jit, static_argnames=("B_seg_len",))
def pallas_concat_heads__softmax_full_mha__memory_aug_recurrent_mem_tr__prompt_kernel(
    A_x: jax.Array,
    A_wqkv: jax.Array,
    A_wo: jax.Array,
    B_x: jax.Array,
    B_mem0: jax.Array,
    B_Wq: jax.Array,
    B_Wk: jax.Array,
    B_Wv: jax.Array,
    B_Wo: jax.Array,
    B_seg_len: int,
):
    _, S, D = A_x.shape
    _, HB, DHB = B_Wq.shape
    M = B_mem0.shape[1]
    SEG = int(B_seg_len)
    L = M + SEG
    G = D // 128
    assert 4 * SEG == TQ and G == 2 * (TQ // SEG)

    vm = pltpu.VMEM
    scratch = [
        vm((S, D), BF16),
        vm((D, 3 * D), BF16),
        vm((D, D), BF16),
        vm((S, D), BF16),
        vm((M, D), BF16),
        vm((G, HB * DHB, 128), BF16),
        vm((2, D // 2, HB, DHB), BF16),
        vm((3, HB, D // 2, DHB), U32),
        vm((G, 64, S), U32),
        vm((G, S // 2, 128), U32),
        vm((G, 64, S), U32),
        vm((S, 4 * TQ), F32),
        vm((S, 4 * TQ), F32),
        vm((8, 4 * TQ), F32),
        vm((8, 4 * TQ), F32),
        vm((64, 4 * TQ), U32),
        vm((64, 4 * TQ), U32),
        vm((G, TQ // 2, 128), U32),
        vm((L, D), F32),
        vm((HB, L, DHB), F32),
        vm((HB, L, DHB), F32),
        vm((HB, L, DHB), F32),
        vm((L, HB * DHB), F32),
        vm((S, 2 * D), BF16),
        pltpu.SemaphoreType.DMA((8,)),
        pltpu.SemaphoreType.DMA((5,)),
        pltpu.SemaphoreType.DMA((2,)),
        pltpu.SemaphoreType.DMA,
        pltpu.SemaphoreType.DMA,
        pltpu.SemaphoreType.DMA,
        pltpu.SemaphoreType.DMA,
    ]
    any_spec = pl.BlockSpec(memory_space=pl.ANY)
    out = pl.pallas_call(
        functools.partial(_kernel, S=S, D=D, HB=HB, DHB=DHB, M=M, SEG=SEG),
        out_shape=jax.ShapeDtypeStruct((S, 2 * D), A_x.dtype),
        in_specs=[any_spec] * 9,
        out_specs=any_spec,
        scratch_shapes=scratch,
        compiler_params=pltpu.CompilerParams(vmem_limit_bytes=120 * 1024 * 1024),
        name="fused_mha_rmt",
    )(
        A_x.reshape(S, D), A_wqkv, A_wo, B_x.reshape(S, D), B_mem0.reshape(M, D),
        B_Wq, B_Wk, B_Wv, B_Wo.reshape(HB * DHB, D),
    )
    return out.reshape(1, S, 2 * D)
```

```python
import functools
import itertools

import jax
import jax.numpy as jnp
from jax import lax
import jax.experimental.pallas as pl
import jax.experimental.pallas.tpu as pltpu

F32 = jnp.float32
BF16 = jnp.bfloat16
U32 = jnp.uint32
LOG2E = 1.4426950408889634
NT_DIMS = (((1,), (1,)), ((), ()))

A_HEADS = 32
TQ = 128
KB = 128
ROWS0 = 512
ROWS1 = 256


def _bf(words):
    return pltpu.bitcast(words, BF16)


def _words(x_f32):
    return pltpu.bitcast(x_f32.astype(BF16), U32)


def _after(never, dep, val):
    return jnp.where(never, dep, val)


def _kernel(
    xa_hbm, wqkv_hbm, woa_hbm, xb_hbm, mem0_hbm, wq_hbm, wk_hbm, wv_hbm, wob_hbm,
    out_hbm,
    xa_s, wqkv_s, woa_s, xb_s, mem0_s, wob_s, raw_s, wb_s,
    qt_s, k_s, vt_s, s0, s1, m0, m1, qs0, qs1, o_s,
    h_s, bq_s, bk_s, bv_s, bo_s, out_s,
    sem_x, sem_w, sem_raw, sem_early, sem_xb, sem_woa, sem_out,
    *, S, D, HB, DHB, M, SEG,
):
    G = D // 128
    DHA = D // A_HEADS
    NJ = S // TQ
    NU = G * NJ
    L = M + SEG
    NR1 = (S - ROWS0) // ROWS1
    DCH = D // 2
    assert NR1 == 6
    SEG_PER_J = TQ // SEG

    x_first = pltpu.make_async_copy(xa_hbm.at[pl.ds(0, ROWS0), :], xa_s.at[pl.ds(0, ROWS0), :], sem_x.at[NR1])

    def x_copy(r):
        rows = pl.ds(ROWS0 + r * ROWS1, ROWS1)
        return pltpu.make_async_copy(xa_hbm.at[rows, :], xa_s.at[rows, :], sem_x.at[r])

    WGRP = [(0, 2), (2, 6), (6, 14), (14, 24)]

    def wqkv_copies(grp):
        lo, hi = WGRP[grp]
        out = []
        n = lo
        while n < hi:
            e = min(hi, (n // G + 1) * G)
            c0 = ((0, 2, 1)[n // G] * G + n % G) * 128
            cols = pl.ds(c0, (e - n) * 128)
            out.append(pltpu.make_async_copy(wqkv_hbm.at[:, cols], wqkv_s.at[:, cols], sem_w.at[grp]))
            n = e
        return out

    def raw_copy(i, half, slot):
        w = (wq_hbm, wk_hbm, wv_hbm)[i]
        return pltpu.make_async_copy(w.at[pl.ds(half * DCH, DCH)], raw_s.at[slot], sem_raw.at[slot])

    def start_raw(c):
        for i in range(3):
            @pl.when(c // 2 == i)
            def _():
                raw_copy(i, c % 2, c % 2).start()

    def wait_raw(c):
        raw_copy(0, 0, c % 2).wait()

    def wob_copy(n):
        return pltpu.make_async_copy(wob_hbm.at[:, pl.ds(n * 128, 128)], wob_s.at[n], sem_early)

    xb_first = pltpu.make_async_copy(xb_hbm.at[pl.ds(0, TQ), :], xb_s.at[pl.ds(0, TQ), :], sem_early)
    xb_rest = pltpu.make_async_copy(xb_hbm.at[pl.ds(TQ, S - TQ), :], xb_s.at[pl.ds(TQ, S - TQ), :], sem_xb)
    mem0_copy = pltpu.make_async_copy(mem0_hbm, mem0_s, sem_early)
    woa_copy = pltpu.make_async_copy(woa_hbm, woa_s, sem_woa)

    wob_w = wob_s.bitcast(U32)

    q_mul = (DHA ** -0.5) * LOG2E
    sub8 = lax.broadcasted_iota(jnp.int32, (8, 128), 0)
    PART_ORDER = (0, 2, 1)
    pieces = [(dd, half) for dd in range(0, DCH, 16) for half in range(HB // 16)]

    def relayout_piece(c, dd, half, gate=None, never=None):
        slot = c % 2
        rows = pl.ds(pl.multiple_of(slot * (DCH // 2) + dd // 2, 8), 8)
        wsel = c // 2
        ev, od = [], []
        for t in range(8):
            a = pltpu.bitcast(raw_s[slot, dd + 2 * t, half * 16:(half + 1) * 16, :], U32)
            b = pltpu.bitcast(raw_s[slot, dd + 2 * t + 1, half * 16:(half + 1) * 16, :], U32)
            if gate is not None:
                a = _after(never, gate, a)
            ev.append((a & U32(0xFFFF)) | (b << 16))
            od.append((a >> 16) | (b & U32(0xFFFF0000)))
        for par, v in ((0, ev), (1, od)):
            for k in (1, 2, 4):
                msk = (sub8 & k) == 0
                nv = list(v)
                for t in range(8):
                    if t & k == 0:
                        x_, y_ = v[t], v[t + k]
                        nv[t] = jnp.where(msk, x_, pltpu.roll(y_, k, 0))
                        nv[t + k] = jnp.where(msk, pltpu.roll(x_, 8 - k, 0), y_)
                v = nv
            for t in range(8):
                wb_s[wsel, 2 * (half * 8 + t) + par, rows, :] = v[t]
        return wb_s[wsel, half * 16 + 15, rows, :]

    def qkv_dots(r0, rows, chunk=None, never=None, hooks=None):
        xt = xa_s[pl.ds(r0, rows), :]
        deps = {}
        gate = None
        npc = len(pieces)
        LAG, GSTEP = 2, 80
        NPS = 3 * G - 2
        for n in range(3 * G):
            if hooks and n in hooks:
                hooks[n]()
            part, g = PART_ORDER[n // G], n % G
            col = part * G + g
            w = wqkv_s[:, col * 128:(col + 1) * 128]
            if n - LAG in deps:
                w = jnp.concatenate([_bf(_after(never, deps[n - LAG], pltpu.bitcast(w[0:16], U32))), w[16:]], axis=0)
            y = jnp.dot(xt, w, preferred_element_type=F32)
            if chunk is not None:
                lo, hi = min(n, NPS) * npc // NPS, min(n + 1, NPS) * npc // NPS
                for t in range(lo, hi):
                    gt = None if gate is None else gate[(t - lo) * GSTEP:(t - lo) * GSTEP + 8]
                    deps[n] = relayout_piece(chunk, *pieces[t], gate=gt, never=never)
            gate = pltpu.bitcast(y, U32)
            if part == 0:
                qt_s[g, :, pl.ds(r0, rows)] = _words((y * q_mul).T)
            elif part == 1:
                k_s[g, pl.ds(pl.multiple_of(r0 // 2, rows // 2), rows // 2), :] = _words(y)
            else:
                vt_s[g, :, pl.ds(r0, rows)] = _words(y.T)

    with jax.named_scope('first'):
        def start(grp):
            for c in wqkv_copies(grp):
                c.start()

        def wait(grp):
            for c in wqkv_copies(grp):
                c.wait()

        x_first.start()
        start(0)
        qs0[...] = jnp.zeros_like(qs0)
        qs1[...] = jnp.zeros_like(qs1)
        x_first.wait()
        wait(0)
        start(1)
        start(2)

        def hook(k):
            def run():
                wait(k)
                if k + 2 < len(WGRP):
                    start(k + 2)
                elif k + 2 == len(WGRP):
                    raw_copy(0, 0, 0).start()
                else:
                    for c in [x_copy(0), wob_copy(6), wob_copy(7), xb_first, mem0_copy]:
                        c.start()
            return run

        qkv_dots(0, ROWS0, hooks={WGRP[k][0]: hook(k) for k in range(1, len(WGRP))})

    def phase1(r, carry):
        wob_copy(r).start()
        x_copy(r).wait()
        wait_raw(r)

        @pl.when(r + 1 < NR1)
        def _():
            x_copy(r + 1).start()

        start_raw(jnp.minimum(r + 1, NR1))

        @pl.when(r == NR1 - 1)
        def _():
            woa_copy.start()

        r0 = pl.multiple_of(ROWS0 + r * ROWS1, ROWS1)
        qkv_dots(r0, ROWS1, chunk=r, never=jnp.full((8, 128), r, jnp.int32) < 0)
        return r

    with jax.named_scope('phase1'):
        lax.fori_loop(0, NR1, phase1, 0)

    S_ = (s0, s1)
    M_ = (m0, m1)
    QS = (qs0, qs1)

    def set_q(u, slot):
        g = u % G
        c0 = pl.multiple_of((u // G) * TQ, TQ)
        for h in range(4):
            QS[slot][h * 16:(h + 1) * 16, h * TQ:(h + 1) * TQ] = qt_s[g, h * 16:(h + 1) * 16, pl.ds(c0, TQ)]

    def scores_block(g, slot, kb, kw=None):
        kw = k_s[g, kb * (KB // 2):(kb + 1) * (KB // 2), :] if kw is None else kw
        sn = jnp.dot(_bf(kw), _bf(QS[slot][...]), preferred_element_type=F32)
        S_[slot][kb * KB:(kb + 1) * KB, :] = sn
        return sn.reshape(KB // 8, 8, 4 * TQ).max(axis=0)

    def finish_max(mrun, slot):
        M_[slot][...] = jnp.broadcast_to(jnp.max(mrun, axis=0, keepdims=True), (8, 4 * TQ))

    def a_slots(u, slot, never):
        un = jnp.minimum(u + 1, NU - 1)
        g = u % G
        cur, nxt = slot, 1 - slot
        set_q(un, nxt)
        m = M_[cur][...]
        mrun = None
        deps = {}
        l = [jnp.zeros((8, TQ), F32) for _ in range(4)]
        acc = [jnp.zeros((DHA, TQ), F32) for _ in range(4)]
        for kb in range(S // KB):
            mx = scores_block(un % G, nxt, kb)
            mrun = mx if mrun is None else jnp.maximum(mrun, mx)
            deps[kb] = mx
            yield
            for h in range(4):
                cols = slice(h * TQ, (h + 1) * TQ)
                mh = m[:, cols]
                if kb - 1 in deps:
                    mh = _after(never, deps[kb - 1][:, cols], mh)
                sc = S_[cur][kb * KB:(kb + 1) * KB, cols]
                p = jnp.exp2(sc.reshape(KB // 8, 8, TQ) - mh[None])
                l[h] = l[h] + p.sum(axis=0)
                vt = _bf(vt_s[g, h * 16:(h + 1) * 16, kb * KB:(kb + 1) * KB])
                acc[h] = acc[h] + jnp.dot(vt, p.reshape(KB, TQ).astype(BF16), preferred_element_type=F32)
            if kb < S // KB - 1:
                yield
        finish_max(mrun, nxt)
        ot = jnp.concatenate(
            [acc[h] / jnp.sum(l[h], axis=0, keepdims=True) for h in range(4)], axis=0)
        o_s[g] = _words(ot.T)
        yield

    scale_b = DHB ** -0.5
    qi = lax.broadcasted_iota(jnp.int32, (L, L), 0)
    ki = lax.broadcasted_iota(jnp.int32, (L, L), 1)
    mask = (qi < M) | (qi >= ki)

    def b_proj(i, h):
        (bq_s, bk_s, bv_s)[i][h] = jnp.dot(h_s[...], _bf(wb_s[i, h]), preferred_element_type=F32)

    def b_scores(h):
        return lax.dot_general(bq_s[h], bk_s[h].astype(BF16), NT_DIMS, preferred_element_type=F32) * scale_b

    def b_softmax_pv(h, s_):
        s_ = jnp.where(mask, s_, -1000000000.0)
        m_ = jnp.max(s_, axis=-1, keepdims=True)
        p_ = jnp.exp(s_ - m_)
        l_ = jnp.sum(p_, axis=-1, keepdims=True)
        r_ = pltpu.reciprocal(l_, approx=True)
        r_ = r_ * (2.0 - l_ * r_)
        bo_s[:, h * DHB:(h + 1) * DHB] = jnp.dot(p_ * r_, bv_s[h].astype(BF16), preferred_element_type=F32)

    def fused_step(s, u0):
        never = jnp.full((8, TQ), s, jnp.int32) < 0
        a_iter = itertools.chain(a_slots(u0, 0, never), a_slots(u0 + 1, 1, never))
        AQ = 29
        LS, LP = 1, 3
        n_a = 0
        r0 = pl.multiple_of(s * SEG, SEG)
        h_s[M:L, :] = xb_s[pl.ds(r0, SEG), :].astype(F32)
        sc, ns, npv = {}, 0, 0
        for t in range(HB):
            has_a = (t + 1) * AQ // HB > t * AQ // HB
            for tok in "qSkavaP":
                if tok in "qkv":
                    b_proj("qkv".index(tok), t)
                elif tok == "a":
                    if has_a:
                        next(a_iter); n_a += 1
                elif tok == "S":
                    if t >= LS:
                        sc[ns] = b_scores(ns); ns += 1
                elif t >= LP:
                    b_softmax_pv(npv, sc.pop(npv)); npv += 1
        for tok in "SAPAPAP":
            if tok == "A":
                next(a_iter); next(a_iter); n_a += 2
            elif tok == "S":
                sc[ns] = b_scores(ns); ns += 1
            else:
                b_softmax_pv(npv, sc.pop(npv)); npv += 1
        assert ns == HB and npv == HB
        assert n_a == 4 * (S // KB)
        mem = []
        for n in range(G):
            a = jnp.dot(bo_s[...], _bf(wob_w[n]), preferred_element_type=F32)
            out_s[pl.ds(r0, SEG), D + n * 128:D + (n + 1) * 128] = a[M:L].astype(BF16)
            mem.append(a[0:M])
        h_s[0:M, :] = jnp.concatenate(mem, axis=1)

    set_q(0, 0)
    mrun = None
    for kb in range(S // KB):
        mx = scores_block(0, 0, kb)
        mrun = mx if mrun is None else jnp.maximum(mrun, mx)
    finish_max(mrun, 0)

    with jax.named_scope('restwait'):
        for c in [wob_copy(n) for n in range(G)] + [xb_first, mem0_copy, woa_copy]:
            c.wait()
        xb_rest.start()
    h_s[0:M, :] = mem0_s[...].astype(F32)

    def out_copy(j, half):
        rows = pl.ds(pl.multiple_of(j * TQ, TQ), TQ)
        cols = pl.ds(half * D, D)
        return pltpu.make_async_copy(out_s.at[rows, cols], out_hbm.at[rows, cols], sem_out)

    def block(j, carry):
        @pl.when(j == 1)
        def _():
            xb_rest.wait()

        def inner(i, c):
            fused_step(j * SEG_PER_J + i, j * G + 2 * i)
            return c

        with jax.named_scope('inner'):
            lax.fori_loop(0, SEG_PER_J, inner, 0)
        out_copy(j, 1).start()

        r0 = pl.multiple_of(j * TQ, TQ)
        ob = jnp.concatenate([_bf(o_s[g]) for g in range(G)], axis=1)
        for n in range(G):
            y = jnp.dot(ob, woa_s[:, n * 128:(n + 1) * 128], preferred_element_type=F32)
            out_s[pl.ds(r0, TQ), n * 128:(n + 1) * 128] = y.astype(BF16)
        out_copy(j, 0).start()
        return carry

    with jax.named_scope('main'):
        lax.fori_loop(0, NJ, block, 0)
    for j in range(NJ):
        out_copy(j, 0).wait()
        out_copy(j, 1).wait()


@functools.partial(jax.jit, static_argnames=("B_seg_len",))
def pallas_concat_heads__softmax_full_mha__memory_aug_recurrent_mem_tr__prompt_kernel(
    A_x: jax.Array,
    A_wqkv: jax.Array,
    A_wo: jax.Array,
    B_x: jax.Array,
    B_mem0: jax.Array,
    B_Wq: jax.Array,
    B_Wk: jax.Array,
    B_Wv: jax.Array,
    B_Wo: jax.Array,
    B_seg_len: int,
):
    _, S, D = A_x.shape
    _, HB, DHB = B_Wq.shape
    M = B_mem0.shape[1]
    SEG = int(B_seg_len)
    L = M + SEG
    G = D // 128
    assert 4 * SEG == TQ and G == 2 * (TQ // SEG)

    vm = pltpu.VMEM
    scratch = [
        vm((S, D), BF16),
        vm((D, 3 * D), BF16),
        vm((D, D), BF16),
        vm((S, D), BF16),
        vm((M, D), BF16),
        vm((G, HB * DHB, 128), BF16),
        vm((2, D // 2, HB, DHB), BF16),
        vm((3, HB, D // 2, DHB), U32),
        vm((G, 64, S), U32),
        vm((G, S // 2, 128), U32),
        vm((G, 64, S), U32),
        vm((S, 4 * TQ), F32),
        vm((S, 4 * TQ), F32),
        vm((8, 4 * TQ), F32),
        vm((8, 4 * TQ), F32),
        vm((64, 4 * TQ), U32),
        vm((64, 4 * TQ), U32),
        vm((G, TQ // 2, 128), U32),
        vm((L, D), F32),
        vm((HB, L, DHB), F32),
        vm((HB, L, DHB), F32),
        vm((HB, L, DHB), F32),
        vm((L, HB * DHB), F32),
        vm((S, 2 * D), BF16),
        pltpu.SemaphoreType.DMA((8,)),
        pltpu.SemaphoreType.DMA((5,)),
        pltpu.SemaphoreType.DMA((2,)),
        pltpu.SemaphoreType.DMA,
        pltpu.SemaphoreType.DMA,
        pltpu.SemaphoreType.DMA,
        pltpu.SemaphoreType.DMA,
    ]
    any_spec = pl.BlockSpec(memory_space=pl.ANY)
    out = pl.pallas_call(
        functools.partial(_kernel, S=S, D=D, HB=HB, DHB=DHB, M=M, SEG=SEG),
        out_shape=jax.ShapeDtypeStruct((S, 2 * D), A_x.dtype),
        in_specs=[any_spec] * 9,
        out_specs=any_spec,
        scratch_shapes=scratch,
        compiler_params=pltpu.CompilerParams(vmem_limit_bytes=120 * 1024 * 1024),
        name="fused_mha_rmt",
    )(
        A_x.reshape(S, D), A_wqkv, A_wo, B_x.reshape(S, D), B_mem0.reshape(M, D),
        B_Wq, B_Wk, B_Wv, B_Wo.reshape(HB * DHB, D),
    )
    return out.reshape(1, S, 2 * D)
```

```python
import functools
import itertools

import jax
import jax.numpy as jnp
from jax import lax
import jax.experimental.pallas as pl
import jax.experimental.pallas.tpu as pltpu

F32 = jnp.float32
BF16 = jnp.bfloat16
U32 = jnp.uint32
LOG2E = 1.4426950408889634
NT_DIMS = (((1,), (1,)), ((), ()))

A_HEADS = 32
TQ = 128
KB = 128
ROWS0 = 512
ROWS1 = 256


def _bf(words):
    return pltpu.bitcast(words, BF16)


def _words(x_f32):
    return pltpu.bitcast(x_f32.astype(BF16), U32)


def _after(never, dep, val):
    return jnp.where(never, dep, val)


def _kernel(
    xa_hbm, wqkv_hbm, woa_hbm, xb_hbm, mem0_hbm, wq_hbm, wk_hbm, wv_hbm, wob_hbm,
    out_hbm,
    xa_s, wqkv_s, woa_s, xb_s, mem0_s, wob_s, raw_s, wb_s,
    qt_s, k_s, vt_s, s0, s1, m0, m1, qs0, qs1, o_s,
    h_s, bq_s, bk_s, bv_s, bo_s, out_s,
    sem_x, sem_w, sem_raw, sem_early, sem_xb, sem_woa, sem_out,
    *, S, D, HB, DHB, M, SEG,
):
    G = D // 128
    DHA = D // A_HEADS
    NJ = S // TQ
    NU = G * NJ
    L = M + SEG
    NR1 = (S - ROWS0) // ROWS1
    DCH = D // 2
    assert NR1 == 6
    SEG_PER_J = TQ // SEG

    x_first = pltpu.make_async_copy(xa_hbm.at[pl.ds(0, ROWS0), :], xa_s.at[pl.ds(0, ROWS0), :], sem_x.at[NR1])

    def x_copy(r):
        rows = pl.ds(ROWS0 + r * ROWS1, ROWS1)
        return pltpu.make_async_copy(xa_hbm.at[rows, :], xa_s.at[rows, :], sem_x.at[r])

    WGRP = [(0, 3), (3, 7), (7, 14), (14, 24)]

    def wqkv_copies(grp):
        lo, hi = WGRP[grp]
        out = []
        n = lo
        while n < hi:
            e = min(hi, (n // G + 1) * G)
            c0 = ((0, 2, 1)[n // G] * G + n % G) * 128
            cols = pl.ds(c0, (e - n) * 128)
            out.append(pltpu.make_async_copy(wqkv_hbm.at[:, cols], wqkv_s.at[:, cols], sem_w.at[grp]))
            n = e
        return out

    def raw_copy(i, half, slot):
        w = (wq_hbm, wk_hbm, wv_hbm)[i]
        return pltpu.make_async_copy(w.at[pl.ds(half * DCH, DCH)], raw_s.at[slot], sem_raw.at[slot])

    def start_raw(c):
        for i in range(3):
            @pl.when(c // 2 == i)
            def _():
                raw_copy(i, c % 2, c % 2).start()

    def wait_raw(c):
        raw_copy(0, 0, c % 2).wait()

    def wob_copy(n):
        return pltpu.make_async_copy(wob_hbm.at[:, pl.ds(n * 128, 128)], wob_s.at[n], sem_early)

    xb_first = pltpu.make_async_copy(xb_hbm.at[pl.ds(0, TQ), :], xb_s.at[pl.ds(0, TQ), :], sem_early)
    xb_rest = pltpu.make_async_copy(xb_hbm.at[pl.ds(TQ, S - TQ), :], xb_s.at[pl.ds(TQ, S - TQ), :], sem_xb)
    mem0_copy = pltpu.make_async_copy(mem0_hbm, mem0_s, sem_early)
    woa_copy = pltpu.make_async_copy(woa_hbm, woa_s, sem_woa)

    wob_w = wob_s.bitcast(U32)

    q_mul = (DHA ** -0.5) * LOG2E
    sub8 = lax.broadcasted_iota(jnp.int32, (8, 128), 0)
    PART_ORDER = (0, 2, 1)
    pieces = [(dd, half) for dd in range(0, DCH, 16) for half in range(HB // 16)]

    def relayout_piece(c, dd, half, gate=None, never=None):
        slot = c % 2
        rows = pl.ds(pl.multiple_of(slot * (DCH // 2) + dd // 2, 8), 8)
        wsel = c // 2
        ev, od = [], []
        for t in range(8):
            a = pltpu.bitcast(raw_s[slot, dd + 2 * t, half * 16:(half + 1) * 16, :], U32)
            b = pltpu.bitcast(raw_s[slot, dd + 2 * t + 1, half * 16:(half + 1) * 16, :], U32)
            if gate is not None:
                a = _after(never, gate, a)
            ev.append((a & U32(0xFFFF)) | (b << 16))
            od.append((a >> 16) | (b & U32(0xFFFF0000)))
        for par, v in ((0, ev), (1, od)):
            for k in (1, 2, 4):
                msk = (sub8 & k) == 0
                nv = list(v)
                for t in range(8):
                    if t & k == 0:
                        x_, y_ = v[t], v[t + k]
                        nv[t] = jnp.where(msk, x_, pltpu.roll(y_, k, 0))
                        nv[t + k] = jnp.where(msk, pltpu.roll(x_, 8 - k, 0), y_)
                v = nv
            for t in range(8):
                wb_s[wsel, 2 * (half * 8 + t) + par, rows, :] = v[t]
        return wb_s[wsel, half * 16 + 15, rows, :]

    def qkv_dots(r0, rows, chunk=None, never=None, hooks=None):
        xt = xa_s[pl.ds(r0, rows), :]
        deps = {}
        gate = None
        npc = len(pieces)
        LAG, GSTEP = 2, 80
        NPS = 3 * G - 2
        pending = []

        def post(part, g, y):
            if part == 0:
                qt_s[g, :, pl.ds(r0, rows)] = _words((y * q_mul).T)
            elif part == 1:
                k_s[g, pl.ds(pl.multiple_of(r0 // 2, rows // 2), rows // 2), :] = _words(y)
            else:
                vt_s[g, :, pl.ds(r0, rows)] = _words(y.T)

        for n in range(3 * G):
            if hooks and n in hooks:
                hooks[n]()
            part, g = PART_ORDER[n // G], n % G
            col = part * G + g
            w = wqkv_s[:, col * 128:(col + 1) * 128]
            if n - LAG in deps:
                w = jnp.concatenate([_bf(_after(never, deps[n - LAG], pltpu.bitcast(w[0:16], U32))), w[16:]], axis=0)
            y = jnp.dot(xt, w, preferred_element_type=F32)
            for it_ in pending:
                post(*it_)
            pending = []
            if chunk is not None:
                lo, hi = min(n, NPS) * npc // NPS, min(n + 1, NPS) * npc // NPS
                for t in range(lo, hi):
                    gt = None if gate is None else gate[(t - lo) * GSTEP:(t - lo) * GSTEP + 8]
                    deps[n] = relayout_piece(chunk, *pieces[t], gate=gt, never=never)
            gate = pltpu.bitcast(y, U32)
            if hooks and n + 1 in hooks:
                pending.append((part, g, y))
            else:
                post(part, g, y)

    with jax.named_scope('first'):
        def start(grp):
            for c in wqkv_copies(grp):
                c.start()

        def wait(grp):
            for c in wqkv_copies(grp):
                c.wait()

        x_first.start()
        start(0)
        qs0[...] = jnp.zeros_like(qs0)
        qs1[...] = jnp.zeros_like(qs1)
        x_first.wait()
        wait(0)
        start(1)
        start(2)

        def hook(k):
            def run():
                wait(k)
                if k + 2 < len(WGRP):
                    start(k + 2)
                elif k + 2 == len(WGRP):
                    raw_copy(0, 0, 0).start()
                else:
                    for c in [x_copy(0), wob_copy(6), wob_copy(7), xb_first, mem0_copy]:
                        c.start()
            return run

        qkv_dots(0, ROWS0, hooks={WGRP[k][0]: hook(k) for k in range(1, len(WGRP))})

    def phase1(r, carry):
        wob_copy(r).start()
        x_copy(r).wait()
        wait_raw(r)

        @pl.when(r + 1 < NR1)
        def _():
            x_copy(r + 1).start()

        start_raw(jnp.minimum(r + 1, NR1))

        @pl.when(r == NR1 - 1)
        def _():
            woa_copy.start()

        r0 = pl.multiple_of(ROWS0 + r * ROWS1, ROWS1)
        qkv_dots(r0, ROWS1, chunk=r, never=jnp.full((8, 128), r, jnp.int32) < 0)
        return r

    with jax.named_scope('phase1'):
        lax.fori_loop(0, NR1, phase1, 0)

    S_ = (s0, s1)
    M_ = (m0, m1)
    QS = (qs0, qs1)

    def set_q(u, slot):
        g = u % G
        c0 = pl.multiple_of((u // G) * TQ, TQ)
        for h in range(4):
            QS[slot][h * 16:(h + 1) * 16, h * TQ:(h + 1) * TQ] = qt_s[g, h * 16:(h + 1) * 16, pl.ds(c0, TQ)]

    def scores_block(g, slot, kb, kw=None):
        kw = k_s[g, kb * (KB // 2):(kb + 1) * (KB // 2), :] if kw is None else kw
        sn = jnp.dot(_bf(kw), _bf(QS[slot][...]), preferred_element_type=F32)
        S_[slot][kb * KB:(kb + 1) * KB, :] = sn
        return sn.reshape(KB // 8, 8, 4 * TQ).max(axis=0)

    def finish_max(mrun, slot):
        M_[slot][...] = jnp.broadcast_to(jnp.max(mrun, axis=0, keepdims=True), (8, 4 * TQ))

    def a_slots(u, slot, never):
        un = jnp.minimum(u + 1, NU - 1)
        g = u % G
        cur, nxt = slot, 1 - slot
        set_q(un, nxt)
        m = M_[cur][...]
        mrun = None
        deps = {}
        l = [jnp.zeros((8, TQ), F32) for _ in range(4)]
        acc = [jnp.zeros((DHA, TQ), F32) for _ in range(4)]
        for kb in range(S // KB):
            mx = scores_block(un % G, nxt, kb)
            mrun = mx if mrun is None else jnp.maximum(mrun, mx)
            deps[kb] = mx
            yield
            for h in range(4):
                cols = slice(h * TQ, (h + 1) * TQ)
                mh = m[:, cols]
                if kb - 1 in deps:
                    mh = _after(never, deps[kb - 1][:, cols], mh)
                sc = S_[cur][kb * KB:(kb + 1) * KB, cols]
                p = jnp.exp2(sc.reshape(KB // 8, 8, TQ) - mh[None])
                l[h] = l[h] + p.sum(axis=0)
                vt = _bf(vt_s[g, h * 16:(h + 1) * 16, kb * KB:(kb + 1) * KB])
                acc[h] = acc[h] + jnp.dot(vt, p.reshape(KB, TQ).astype(BF16), preferred_element_type=F32)
            if kb < S // KB - 1:
                yield
        finish_max(mrun, nxt)
        ot = jnp.concatenate(
            [acc[h] / jnp.sum(l[h], axis=0, keepdims=True) for h in range(4)], axis=0)
        o_s[g] = _words(ot.T)
        yield

    scale_b = DHB ** -0.5
    qi = lax.broadcasted_iota(jnp.int32, (L, L), 0)
    ki = lax.broadcasted_iota(jnp.int32, (L, L), 1)
    mask = (qi < M) | (qi >= ki)

    def b_proj(i, h):
        (bq_s, bk_s, bv_s)[i][h] = jnp.dot(h_s[...], _bf(wb_s[i, h]), preferred_element_type=F32)

    def b_scores(h):
        return lax.dot_general(bq_s[h], bk_s[h].astype(BF16), NT_DIMS, preferred_element_type=F32) * scale_b

    def b_softmax_pv(h, s_):
        s_ = jnp.where(mask, s_, -1000000000.0)
        m_ = jnp.max(s_, axis=-1, keepdims=True)
        p_ = jnp.exp(s_ - m_)
        l_ = jnp.sum(p_, axis=-1, keepdims=True)
        r_ = pltpu.reciprocal(l_, approx=True)
        r_ = r_ * (2.0 - l_ * r_)
        bo_s[:, h * DHB:(h + 1) * DHB] = jnp.dot(p_ * r_, bv_s[h].astype(BF16), preferred_element_type=F32)

    def fused_step(s, u0):
        never = jnp.full((8, TQ), s, jnp.int32) < 0
        a_iter = itertools.chain(a_slots(u0, 0, never), a_slots(u0 + 1, 1, never))
        AQ = 29
        LS, LP = 1, 3
        n_a = 0
        r0 = pl.multiple_of(s * SEG, SEG)
        h_s[M:L, :] = xb_s[pl.ds(r0, SEG), :].astype(F32)
        sc, ns, npv = {}, 0, 0
        for t in range(HB):
            has_a = (t + 1) * AQ // HB > t * AQ // HB
            for tok in "qSkavaP":
                if tok in "qkv":
                    b_proj("qkv".index(tok), t)
                elif tok == "a":
                    if has_a:
                        next(a_iter); n_a += 1
                elif tok == "S":
                    if t >= LS:
                        sc[ns] = b_scores(ns); ns += 1
                elif t >= LP:
                    b_softmax_pv(npv, sc.pop(npv)); npv += 1
        for tok in "SAPAPAP":
            if tok == "A":
                next(a_iter); next(a_iter); n_a += 2
            elif tok == "S":
                sc[ns] = b_scores(ns); ns += 1
            else:
                b_softmax_pv(npv, sc.pop(npv)); npv += 1
        assert ns == HB and npv == HB
        assert n_a == 4 * (S // KB)
        mem = []
        for n in range(G):
            a = jnp.dot(bo_s[...], _bf(wob_w[n]), preferred_element_type=F32)
            out_s[pl.ds(r0, SEG), D + n * 128:D + (n + 1) * 128] = a[M:L].astype(BF16)
            mem.append(a[0:M])
        h_s[0:M, :] = jnp.concatenate(mem, axis=1)

    set_q(0, 0)
    mrun = None
    for kb in range(S // KB):
        mx = scores_block(0, 0, kb)
        mrun = mx if mrun is None else jnp.maximum(mrun, mx)
    finish_max(mrun, 0)

    with jax.named_scope('restwait'):
        for c in [wob_copy(n) for n in range(G)] + [xb_first, mem0_copy, woa_copy]:
            c.wait()
        xb_rest.start()
    h_s[0:M, :] = mem0_s[...].astype(F32)

    def out_copy(j, half):
        rows = pl.ds(pl.multiple_of(j * TQ, TQ), TQ)
        cols = pl.ds(half * D, D)
        return pltpu.make_async_copy(out_s.at[rows, cols], out_hbm.at[rows, cols], sem_out)

    def block(j, carry):
        @pl.when(j == 1)
        def _():
            xb_rest.wait()

        def inner(i, c):
            fused_step(j * SEG_PER_J + i, j * G + 2 * i)
            return c

        with jax.named_scope('inner'):
            lax.fori_loop(0, SEG_PER_J, inner, 0)
        out_copy(j, 1).start()

        r0 = pl.multiple_of(j * TQ, TQ)
        ob = jnp.concatenate([_bf(o_s[g]) for g in range(G)], axis=1)
        for n in range(G):
            y = jnp.dot(ob, woa_s[:, n * 128:(n + 1) * 128], preferred_element_type=F32)
            out_s[pl.ds(r0, TQ), n * 128:(n + 1) * 128] = y.astype(BF16)
        out_copy(j, 0).start()
        return carry

    with jax.named_scope('main'):
        lax.fori_loop(0, NJ, block, 0)
    for j in range(NJ):
        out_copy(j, 0).wait()
        out_copy(j, 1).wait()


@functools.partial(jax.jit, static_argnames=("B_seg_len",))
def pallas_concat_heads__softmax_full_mha__memory_aug_recurrent_mem_tr__prompt_kernel(
    A_x: jax.Array,
    A_wqkv: jax.Array,
    A_wo: jax.Array,
    B_x: jax.Array,
    B_mem0: jax.Array,
    B_Wq: jax.Array,
    B_Wk: jax.Array,
    B_Wv: jax.Array,
    B_Wo: jax.Array,
    B_seg_len: int,
):
    _, S, D = A_x.shape
    _, HB, DHB = B_Wq.shape
    M = B_mem0.shape[1]
    SEG = int(B_seg_len)
    L = M + SEG
    G = D // 128
    assert 4 * SEG == TQ and G == 2 * (TQ // SEG)

    vm = pltpu.VMEM
    scratch = [
        vm((S, D), BF16),
        vm((D, 3 * D), BF16),
        vm((D, D), BF16),
        vm((S, D), BF16),
        vm((M, D), BF16),
        vm((G, HB * DHB, 128), BF16),
        vm((2, D // 2, HB, DHB), BF16),
        vm((3, HB, D // 2, DHB), U32),
        vm((G, 64, S), U32),
        vm((G, S // 2, 128), U32),
        vm((G, 64, S), U32),
        vm((S, 4 * TQ), F32),
        vm((S, 4 * TQ), F32),
        vm((8, 4 * TQ), F32),
        vm((8, 4 * TQ), F32),
        vm((64, 4 * TQ), U32),
        vm((64, 4 * TQ), U32),
        vm((G, TQ // 2, 128), U32),
        vm((L, D), F32),
        vm((HB, L, DHB), F32),
        vm((HB, L, DHB), F32),
        vm((HB, L, DHB), F32),
        vm((L, HB * DHB), F32),
        vm((S, 2 * D), BF16),
        pltpu.SemaphoreType.DMA((8,)),
        pltpu.SemaphoreType.DMA((5,)),
        pltpu.SemaphoreType.DMA((2,)),
        pltpu.SemaphoreType.DMA,
        pltpu.SemaphoreType.DMA,
        pltpu.SemaphoreType.DMA,
        pltpu.SemaphoreType.DMA,
    ]
    any_spec = pl.BlockSpec(memory_space=pl.ANY)
    out = pl.pallas_call(
        functools.partial(_kernel, S=S, D=D, HB=HB, DHB=DHB, M=M, SEG=SEG),
        out_shape=jax.ShapeDtypeStruct((S, 2 * D), A_x.dtype),
        in_specs=[any_spec] * 9,
        out_specs=any_spec,
        scratch_shapes=scratch,
        compiler_params=pltpu.CompilerParams(vmem_limit_bytes=120 * 1024 * 1024),
        name="fused_mha_rmt",
    )(
        A_x.reshape(S, D), A_wqkv, A_wo, B_x.reshape(S, D), B_mem0.reshape(M, D),
        B_Wq, B_Wk, B_Wv, B_Wo.reshape(HB * DHB, D),
    )
    return out.reshape(1, S, 2 * D)
```

```python
import functools
import itertools

import jax
import jax.numpy as jnp
from jax import lax
import jax.experimental.pallas as pl
import jax.experimental.pallas.tpu as pltpu

F32 = jnp.float32
BF16 = jnp.bfloat16
U32 = jnp.uint32
LOG2E = 1.4426950408889634
NT_DIMS = (((1,), (1,)), ((), ()))

A_HEADS = 32
TQ = 128
KB = 128
ROWS0 = 512
ROWS1 = 256


def _bf(words):
    return pltpu.bitcast(words, BF16)


def _words(x_f32):
    return pltpu.bitcast(x_f32.astype(BF16), U32)


def _after(never, dep, val):
    return jnp.where(never, dep, val)


def _kernel(
    xa_hbm, wqkv_hbm, woa_hbm, xb_hbm, mem0_hbm, wq_hbm, wk_hbm, wv_hbm, wob_hbm,
    out_hbm,
    xa_s, wqkv_s, woa_s, xb_s, mem0_s, wob_s, raw_s, wb_s,
    qt_s, k_s, vt_s, s0, s1, m0, m1, qs0, qs1, o_s,
    h_s, bq_s, bk_s, bv_s, bo_s, out_s,
    sem_x, sem_w, sem_raw, sem_early, sem_xb, sem_woa, sem_out,
    *, S, D, HB, DHB, M, SEG,
):
    G = D // 128
    DHA = D // A_HEADS
    NJ = S // TQ
    NU = G * NJ
    L = M + SEG
    NR1 = (S - ROWS0) // ROWS1
    DCH = D // 2
    assert NR1 == 6
    SEG_PER_J = TQ // SEG

    x_first = pltpu.make_async_copy(xa_hbm.at[pl.ds(0, ROWS0), :], xa_s.at[pl.ds(0, ROWS0), :], sem_x.at[NR1])

    def x_copy(r):
        rows = pl.ds(ROWS0 + r * ROWS1, ROWS1)
        return pltpu.make_async_copy(xa_hbm.at[rows, :], xa_s.at[rows, :], sem_x.at[r])

    WGRP = [(0, 3), (3, 7), (7, 14), (14, 24)]

    def wqkv_copies(grp):
        lo, hi = WGRP[grp]
        out = []
        n = lo
        while n < hi:
            e = min(hi, (n // G + 1) * G)
            c0 = ((0, 2, 1)[n // G] * G + n % G) * 128
            cols = pl.ds(c0, (e - n) * 128)
            out.append(pltpu.make_async_copy(wqkv_hbm.at[:, cols], wqkv_s.at[:, cols], sem_w.at[grp]))
            n = e
        return out

    def raw_copy(i, half, slot):
        w = (wq_hbm, wk_hbm, wv_hbm)[i]
        return pltpu.make_async_copy(w.at[pl.ds(half * DCH, DCH)], raw_s.at[slot], sem_raw.at[slot])

    def start_raw(c):
        for i in range(3):
            @pl.when(c // 2 == i)
            def _():
                raw_copy(i, c % 2, c % 2).start()

    def wait_raw(c):
        raw_copy(0, 0, c % 2).wait()

    def wob_copy(n):
        return pltpu.make_async_copy(wob_hbm.at[:, pl.ds(n * 128, 128)], wob_s.at[n], sem_early)

    xb_first = pltpu.make_async_copy(xb_hbm.at[pl.ds(0, TQ), :], xb_s.at[pl.ds(0, TQ), :], sem_early)
    xb_rest = pltpu.make_async_copy(xb_hbm.at[pl.ds(TQ, S - TQ), :], xb_s.at[pl.ds(TQ, S - TQ), :], sem_xb)
    mem0_copy = pltpu.make_async_copy(mem0_hbm, mem0_s, sem_early)
    woa_copy = pltpu.make_async_copy(woa_hbm, woa_s, sem_woa)

    wob_w = wob_s.bitcast(U32)

    q_mul = (DHA ** -0.5) * LOG2E
    sub8 = lax.broadcasted_iota(jnp.int32, (8, 128), 0)
    PART_ORDER = (0, 2, 1)
    pieces = [(dd, half) for dd in range(0, DCH, 16) for half in range(HB // 16)]

    def relayout_piece(c, dd, half, gate=None, never=None):
        slot = c % 2
        rows = pl.ds(pl.multiple_of(slot * (DCH // 2) + dd // 2, 8), 8)
        wsel = c // 2
        ev, od = [], []
        for t in range(8):
            a = pltpu.bitcast(raw_s[slot, dd + 2 * t, half * 16:(half + 1) * 16, :], U32)
            b = pltpu.bitcast(raw_s[slot, dd + 2 * t + 1, half * 16:(half + 1) * 16, :], U32)
            if gate is not None:
                a = _after(never, gate, a)
            ev.append((a & U32(0xFFFF)) | (b << 16))
            od.append((a >> 16) | (b & U32(0xFFFF0000)))
        for par, v in ((0, ev), (1, od)):
            for k in (1, 2, 4):
                msk = (sub8 & k) == 0
                nv = list(v)
                for t in range(8):
                    if t & k == 0:
                        x_, y_ = v[t], v[t + k]
                        nv[t] = jnp.where(msk, x_, pltpu.roll(y_, k, 0))
                        nv[t + k] = jnp.where(msk, pltpu.roll(x_, 8 - k, 0), y_)
                v = nv
            for t in range(8):
                wb_s[wsel, 2 * (half * 8 + t) + par, rows, :] = v[t]
        return wb_s[wsel, half * 16 + 15, rows, :]

    def qkv_dots(r0, rows, chunk=None, never=None, hooks=None):
        xt = xa_s[pl.ds(r0, rows), :]
        deps = {}
        gate = None
        npc = len(pieces)
        LAG, GSTEP = 2, 80
        NPS = 3 * G - 2
        pending = []

        def post(part, g, y):
            if part == 0:
                qt_s[g, :, pl.ds(r0, rows)] = _words((y * q_mul).T)
            elif part == 1:
                k_s[g, pl.ds(pl.multiple_of(r0 // 2, rows // 2), rows // 2), :] = _words(y)
            else:
                vt_s[g, :, pl.ds(r0, rows)] = _words(y.T)

        for n in range(3 * G):
            if hooks and n in hooks:
                hooks[n]()
            part, g = PART_ORDER[n // G], n % G
            col = part * G + g
            w = wqkv_s[:, col * 128:(col + 1) * 128]
            if n - LAG in deps:
                w = jnp.concatenate([_bf(_after(never, deps[n - LAG], pltpu.bitcast(w[0:16], U32))), w[16:]], axis=0)
            y = jnp.dot(xt, w, preferred_element_type=F32)
            for it_ in pending:
                post(*it_)
            pending = []
            if chunk is not None:
                lo, hi = min(n, NPS) * npc // NPS, min(n + 1, NPS) * npc // NPS
                for t in range(lo, hi):
                    gt = None if gate is None else gate[(t - lo) * GSTEP:(t - lo) * GSTEP + 8]
                    deps[n] = relayout_piece(chunk, *pieces[t], gate=gt, never=never)
            gate = pltpu.bitcast(y, U32)
            if hooks and n + 1 in hooks:
                pending.append((part, g, y))
            else:
                post(part, g, y)

    def start(grp):
        for c in wqkv_copies(grp):
            c.start()

    def wait(grp):
        for c in wqkv_copies(grp):
            c.wait()

    x_first.start()
    start(0)
    qs0[...] = jnp.zeros_like(qs0)
    qs1[...] = jnp.zeros_like(qs1)
    x_first.wait()
    wait(0)
    start(1)
    start(2)

    def hook(k):
        def run():
            wait(k)
            if k + 2 < len(WGRP):
                start(k + 2)
            elif k + 2 == len(WGRP):
                raw_copy(0, 0, 0).start()
            else:
                for c in [x_copy(0), wob_copy(6), wob_copy(7), xb_first, mem0_copy]:
                    c.start()
        return run

    qkv_dots(0, ROWS0, hooks={WGRP[k][0]: hook(k) for k in range(1, len(WGRP))})

    def phase1(r, carry):
        wob_copy(r).start()
        x_copy(r).wait()
        wait_raw(r)

        @pl.when(r + 1 < NR1)
        def _():
            x_copy(r + 1).start()

        start_raw(jnp.minimum(r + 1, NR1))

        @pl.when(r == NR1 - 1)
        def _():
            woa_copy.start()

        r0 = pl.multiple_of(ROWS0 + r * ROWS1, ROWS1)
        qkv_dots(r0, ROWS1, chunk=r, never=jnp.full((8, 128), r, jnp.int32) < 0)
        return r

    lax.fori_loop(0, NR1, phase1, 0)

    S_ = (s0, s1)
    M_ = (m0, m1)
    QS = (qs0, qs1)

    def set_q(u, slot):
        g = u % G
        c0 = pl.multiple_of((u // G) * TQ, TQ)
        for h in range(4):
            QS[slot][h * 16:(h + 1) * 16, h * TQ:(h + 1) * TQ] = qt_s[g, h * 16:(h + 1) * 16, pl.ds(c0, TQ)]

    def scores_block(g, slot, kb, kw=None):
        kw = k_s[g, kb * (KB // 2):(kb + 1) * (KB // 2), :] if kw is None else kw
        sn = jnp.dot(_bf(kw), _bf(QS[slot][...]), preferred_element_type=F32)
        S_[slot][kb * KB:(kb + 1) * KB, :] = sn
        return sn.reshape(KB // 8, 8, 4 * TQ).max(axis=0)

    def finish_max(mrun, slot):
        M_[slot][...] = jnp.broadcast_to(jnp.max(mrun, axis=0, keepdims=True), (8, 4 * TQ))

    def a_slots(u, slot, never):
        un = jnp.minimum(u + 1, NU - 1)
        g = u % G
        cur, nxt = slot, 1 - slot
        set_q(un, nxt)
        m = M_[cur][...]
        mrun = None
        deps = {}
        l = [jnp.zeros((8, TQ), F32) for _ in range(4)]
        acc = [jnp.zeros((DHA, TQ), F32) for _ in range(4)]
        for kb in range(S // KB):
            mx = scores_block(un % G, nxt, kb)
            mrun = mx if mrun is None else jnp.maximum(mrun, mx)
            deps[kb] = mx
            yield
            for h in range(4):
                cols = slice(h * TQ, (h + 1) * TQ)
                mh = m[:, cols]
                if kb - 1 in deps:
                    mh = _after(never, deps[kb - 1][:, cols], mh)
                sc = S_[cur][kb * KB:(kb + 1) * KB, cols]
                p = jnp.exp2(sc.reshape(KB // 8, 8, TQ) - mh[None])
                l[h] = l[h] + p.sum(axis=0)
                vt = _bf(vt_s[g, h * 16:(h + 1) * 16, kb * KB:(kb + 1) * KB])
                acc[h] = acc[h] + jnp.dot(vt, p.reshape(KB, TQ).astype(BF16), preferred_element_type=F32)
            if kb < S // KB - 1:
                yield
        finish_max(mrun, nxt)
        ot = jnp.concatenate(
            [acc[h] / jnp.sum(l[h], axis=0, keepdims=True) for h in range(4)], axis=0)
        o_s[g] = _words(ot.T)
        yield

    scale_b = DHB ** -0.5
    qi = lax.broadcasted_iota(jnp.int32, (L, L), 0)
    ki = lax.broadcasted_iota(jnp.int32, (L, L), 1)
    mask = (qi < M) | (qi >= ki)

    def b_proj(i, h):
        (bq_s, bk_s, bv_s)[i][h] = jnp.dot(h_s[...], _bf(wb_s[i, h]), preferred_element_type=F32)

    def b_scores(h):
        return lax.dot_general(bq_s[h], bk_s[h].astype(BF16), NT_DIMS, preferred_element_type=F32) * scale_b

    def b_softmax_pv(h, s_):
        s_ = jnp.where(mask, s_, -1000000000.0)
        m_ = jnp.max(s_, axis=-1, keepdims=True)
        p_ = jnp.exp(s_ - m_)
        l_ = jnp.sum(p_, axis=-1, keepdims=True)
        r_ = pltpu.reciprocal(l_, approx=True)
        r_ = r_ * (2.0 - l_ * r_)
        bo_s[:, h * DHB:(h + 1) * DHB] = jnp.dot(p_ * r_, bv_s[h].astype(BF16), preferred_element_type=F32)

    def fused_step(s, u0):
        never = jnp.full((8, TQ), s, jnp.int32) < 0
        a_iter = itertools.chain(a_slots(u0, 0, never), a_slots(u0 + 1, 1, never))
        AQ = 29
        LS, LP = 1, 3
        n_a = 0
        r0 = pl.multiple_of(s * SEG, SEG)
        h_s[M:L, :] = xb_s[pl.ds(r0, SEG), :].astype(F32)
        sc, ns, npv = {}, 0, 0
        for t in range(HB):
            has_a = (t + 1) * AQ // HB > t * AQ // HB
            for tok in "qSkavaP":
                if tok in "qkv":
                    b_proj("qkv".index(tok), t)
                elif tok == "a":
                    if has_a:
                        next(a_iter); n_a += 1
                elif tok == "S":
                    if t >= LS:
                        sc[ns] = b_scores(ns); ns += 1
                elif t >= LP:
                    b_softmax_pv(npv, sc.pop(npv)); npv += 1
        for tok in "aSaaPaPaaP":
            if tok == "a":
                next(a_iter); n_a += 1
            elif tok == "S":
                sc[ns] = b_scores(ns); ns += 1
            else:
                b_softmax_pv(npv, sc.pop(npv)); npv += 1
        assert ns == HB and npv == HB
        assert n_a == 4 * (S // KB)
        mem = []
        for n in range(G):
            a = jnp.dot(bo_s[...], _bf(wob_w[n]), preferred_element_type=F32)
            out_s[pl.ds(r0, SEG), D + n * 128:D + (n + 1) * 128] = a[M:L].astype(BF16)
            mem.append(a[0:M])
        h_s[0:M, :] = jnp.concatenate(mem, axis=1)

    set_q(0, 0)
    mrun = None
    for kb in range(S // KB):
        mx = scores_block(0, 0, kb)
        mrun = mx if mrun is None else jnp.maximum(mrun, mx)
    finish_max(mrun, 0)

    for c in [wob_copy(n) for n in range(G)] + [xb_first, mem0_copy, woa_copy]:
        c.wait()
    xb_rest.start()
    h_s[0:M, :] = mem0_s[...].astype(F32)

    def out_copy(j, half):
        rows = pl.ds(pl.multiple_of(j * TQ, TQ), TQ)
        cols = pl.ds(half * D, D)
        return pltpu.make_async_copy(out_s.at[rows, cols], out_hbm.at[rows, cols], sem_out)

    def block(j, carry):
        @pl.when(j == 1)
        def _():
            xb_rest.wait()

        def inner(i, c):
            fused_step(j * SEG_PER_J + i, j * G + 2 * i)
            return c

        lax.fori_loop(0, SEG_PER_J, inner, 0)
        out_copy(j, 1).start()

        r0 = pl.multiple_of(j * TQ, TQ)
        ob = jnp.concatenate([_bf(o_s[g]) for g in range(G)], axis=1)
        for n in range(G):
            y = jnp.dot(ob, woa_s[:, n * 128:(n + 1) * 128], preferred_element_type=F32)
            out_s[pl.ds(r0, TQ), n * 128:(n + 1) * 128] = y.astype(BF16)
        out_copy(j, 0).start()
        return carry

    lax.fori_loop(0, NJ, block, 0)
    for j in range(NJ):
        out_copy(j, 0).wait()
        out_copy(j, 1).wait()


@functools.partial(jax.jit, static_argnames=("B_seg_len",))
def pallas_concat_heads__softmax_full_mha__memory_aug_recurrent_mem_tr__prompt_kernel(
    A_x: jax.Array,
    A_wqkv: jax.Array,
    A_wo: jax.Array,
    B_x: jax.Array,
    B_mem0: jax.Array,
    B_Wq: jax.Array,
    B_Wk: jax.Array,
    B_Wv: jax.Array,
    B_Wo: jax.Array,
    B_seg_len: int,
):
    _, S, D = A_x.shape
    _, HB, DHB = B_Wq.shape
    M = B_mem0.shape[1]
    SEG = int(B_seg_len)
    L = M + SEG
    G = D // 128
    assert 4 * SEG == TQ and G == 2 * (TQ // SEG)

    vm = pltpu.VMEM
    scratch = [
        vm((S, D), BF16),
        vm((D, 3 * D), BF16),
        vm((D, D), BF16),
        vm((S, D), BF16),
        vm((M, D), BF16),
        vm((G, HB * DHB, 128), BF16),
        vm((2, D // 2, HB, DHB), BF16),
        vm((3, HB, D // 2, DHB), U32),
        vm((G, 64, S), U32),
        vm((G, S // 2, 128), U32),
        vm((G, 64, S), U32),
        vm((S, 4 * TQ), F32),
        vm((S, 4 * TQ), F32),
        vm((8, 4 * TQ), F32),
        vm((8, 4 * TQ), F32),
        vm((64, 4 * TQ), U32),
        vm((64, 4 * TQ), U32),
        vm((G, TQ // 2, 128), U32),
        vm((L, D), F32),
        vm((HB, L, DHB), F32),
        vm((HB, L, DHB), F32),
        vm((HB, L, DHB), F32),
        vm((L, HB * DHB), F32),
        vm((S, 2 * D), BF16),
        pltpu.SemaphoreType.DMA((7,)),
        pltpu.SemaphoreType.DMA((4,)),
        pltpu.SemaphoreType.DMA((2,)),
        pltpu.SemaphoreType.DMA,
        pltpu.SemaphoreType.DMA,
        pltpu.SemaphoreType.DMA,
        pltpu.SemaphoreType.DMA,
    ]
    any_spec = pl.BlockSpec(memory_space=pl.ANY)
    out = pl.pallas_call(
        functools.partial(_kernel, S=S, D=D, HB=HB, DHB=DHB, M=M, SEG=SEG),
        out_shape=jax.ShapeDtypeStruct((S, 2 * D), A_x.dtype),
        in_specs=[any_spec] * 9,
        out_specs=any_spec,
        scratch_shapes=scratch,
        compiler_params=pltpu.CompilerParams(vmem_limit_bytes=120 * 1024 * 1024),
        name="fused_mha_rmt",
    )(
        A_x.reshape(S, D), A_wqkv, A_wo, B_x.reshape(S, D), B_mem0.reshape(M, D),
        B_Wq, B_Wk, B_Wv, B_Wo.reshape(HB * DHB, D),
    )
    return out.reshape(1, S, 2 * D)
```
